```python
import os as _os
_os.environ.setdefault("JAX_PLATFORMS", "cpu")
import jax
import jax.numpy as jnp

def _softmax(x, axis=-1):
    return jax.nn.softmax(x, axis=axis)
def _gelu(x):
    return jax.nn.gelu(x, approximate=True)
def _silu(x):
    return jax.nn.silu(x)
def _sigmoid(x):
    return jax.nn.sigmoid(x)
def _layernorm(x, axis=-1, eps=1e-5):
    m = jnp.mean(x, axis=axis, keepdims=True)
    v = jnp.var(x, axis=axis, keepdims=True)
    return (x - m) / jnp.sqrt(v + eps)
def _scatter_add(tgt, idx, src, axis=0):
    return tgt.at[idx].add(src)
def _segment_sum(src, seg, n):
    return jax.ops.segment_sum(src, seg, n)
class _Rng:
    def __init__(self, key):
        self._k = key
    def _next(self):
        self._k, sub = jax.random.split(self._k)
        return sub
    def normal(self, shape):
        return jax.random.normal(self._next(), shape, dtype=jnp.bfloat16)
    def randint(self, lo, hi, shape):
        return jax.random.randint(self._next(), shape, lo, hi, dtype=jnp.int32)
    def uniform(self, shape, lo=0.0, hi=1.0):
        return jax.random.uniform(self._next(), shape, jnp.bfloat16, lo, hi)
    def permutation(self, n):
        return jax.random.permutation(self._next(), n)


kernel_name = 'standalone__mha_block_cached__near_ridge'

def setup_inputs():
    _rng = _Rng(jax.random.key(int.from_bytes(__import__("os").urandom(4), "little")))
    _w = (lambda a: (lambda t: t.astype(jnp.bfloat16) if jnp.issubdtype(t.dtype, jnp.floating) else t)(jnp.asarray(a)))
    B, Sq, D = 8, 144, 448
    H, Sk, Dh = 16, 2048, 256
    return {
        "x": _w((lambda *s: _rng.normal(s) * 0.8)(B, Sq, D)),
        "k_cache": _w((lambda *s: _rng.normal(s) * 0.8)(B, H, Sk, Dh)),
        "v_cache": _w((lambda *s: _rng.normal(s) * 0.05)(B, H, Sk, Dh)),
        "wq": _w((lambda *s: _rng.normal(s) * 0.8)(D, H * Dh) * (D ** -0.5)),
        "wo": _w((lambda *s: _rng.normal(s) * 0.05)(H * Dh, D) * ((H * Dh) ** -0.5)),
    }

def reference(x, k_cache, v_cache, wq, wo):
    B, Sq, D = x.shape
    H, Dh = 16, 256
    q = (lambda x, *d: x.transpose(*d))((x @ wq).reshape(B, Sq, H, Dh), 0, 2, 1, 3)
    scores = jnp.einsum("bhqd,bhkd->bhqk", q, k_cache) * (Dh ** -0.5)
    p = _softmax(scores, axis=-1)
    o = jnp.einsum("bhqk,bhkd->bhqd", p, v_cache)
    return (lambda x, *d: x.transpose(*d))(o, 0, 2, 1, 3).reshape(B, Sq, H * Dh) @ wo
```

```python
import jax, jax.numpy as jnp
from jax import lax
from jax.experimental import pallas as pl
from jax.experimental.pallas import tpu as pltpu

NT = (((1,), (1,)), ((), ()))
F32 = jnp.float32
BF = jnp.bfloat16

def make(TB=None, TI=None, DELAY=95, scopes=False, TL=None, defer=True, lo_at=3):
    TB = TB or [80] * 20
    TI = TI if TI is not None else [96, 96, 96, 80, 80]
    TL = TL or [112] * 8 + [96] * 12
    NVB = 3
    NC = 8
    WS = 64
    def kern(x_hbm, k_hbm, v_hbm, wq_hbm, wot_hbm, o_hbm,
             x_buf, big, s_ref, m_ref, acc_ref, o_buf,
             ksem, vsem, wsem, xsem, osem):
        B, Sq, D = x_hbm.shape
        _, H, Sk, Dh = k_hbm.shape
        N = B * H
        CK = Sk // NC
        assert sum(TB) + sum(TI) == Sk and sum(TL) == Sk and len(TB) == 20
        assert D // WS == B - 1
        K0 = 0
        V0 = 2 * Sk
        WQ0 = V0 + NVB * Sk
        WO0 = WQ0 + 2 * D
        P0 = WO0 + 2 * D
        def al(v):
            return pl.multiple_of(v, 64)
        def krow(n): return al(K0 + lax.rem(n, 2) * Sk)
        def vrow(n): return al(V0 + lax.rem(n, NVB) * Sk)
        def wqrow(h): return al(WQ0 + lax.rem(h, 2) * D)
        def worow(h): return al(WO0 + lax.rem(h, 2) * D)
        hd = lambda n: lax.div(n, B)
        bt = lambda n: lax.rem(n, B)

        def k_part(n, r0, cnt):
            return pltpu.make_async_copy(k_hbm.at[bt(n), hd(n), pl.ds(r0, cnt)],
                                         big.at[pl.ds(pl.multiple_of(krow(n) + r0, 16), cnt)], ksem.at[lax.rem(n, 2)])
        def v_cp(n):
            return pltpu.make_async_copy(v_hbm.at[bt(n), hd(n)], big.at[pl.ds(vrow(n), Sk)], vsem.at[lax.rem(n, NVB)])
        def wq_cp(h, r0, cnt):
            return pltpu.make_async_copy(wq_hbm.at[pl.ds(r0, cnt), pl.ds(pl.multiple_of(h * Dh, Dh), Dh)],
                                         big.at[pl.ds(al(wqrow(h) + r0), cnt)], wsem.at[0])
        def wo_cp(h, r0, cnt):
            return pltpu.make_async_copy(wot_hbm.at[pl.ds(r0, cnt), pl.ds(pl.multiple_of(h * Dh, Dh), Dh)],
                                         big.at[pl.ds(al(worow(h) + r0), cnt)], wsem.at[1])
        def x_cp(b):
            return pltpu.make_async_copy(x_hbm.at[b], x_buf.at[b], xsem.at[b])
        def o_cp(b0, cnt, s):
            return pltpu.make_async_copy(o_buf.at[pl.ds(b0, cnt)], o_hbm.at[pl.ds(b0, cnt)], osem.at[s])

        def prow(j):
            return pl.ds(P0 + j * Sq, Sq)

        def stage_abc(n, tick, do_ab, do_c):
            if do_ab:
                x = x_buf[bt(n)]
                qs = []
                for c in range(2):
                    tick()
                    w = big[pl.ds(wqrow(hd(n)), D), pl.ds(c * 128, 128)]
                    qs.append(jnp.dot(x, w, preferred_element_type=F32))
                q = (jnp.concatenate(qs, axis=1) * (Dh ** -0.5)).astype(BF)
            if do_c:
                m_old = m_ref[...]
            m = None
            l = None
            for j in range(NC):
                if do_c:
                    sa = s_ref[:, pl.ds(j * CK, 128)]
                    sb = s_ref[:, pl.ds(j * CK + 128, 128)]
                if do_ab:
                    tick()
                    kj = big[pl.ds(al(krow(n) + j * CK), CK), :]
                if do_c:
                    pa = jnp.exp(sa - m_old)
                    pb = jnp.exp(sb - m_old)
                    lj = pa + pb
                    l = lj if l is None else l + lj
                    big[prow(j), :] = jnp.concatenate([pa, pb], axis=1).astype(BF)
                if do_ab:
                    sj = lax.dot_general(q, kj, NT, preferred_element_type=F32)
                    s_ref[:, pl.ds(j * CK, CK)] = sj
                    mj = jnp.maximum(sj[:, :128], sj[:, 128:])
                    m = mj if m is None else jnp.maximum(m, mj)
            if do_ab:
                m_ref[...] = jnp.broadcast_to(jnp.max(m, axis=-1, keepdims=True), m_ref.shape)
            if do_c:
                return jnp.sum(l, axis=-1, keepdims=True)

        def stage_de(n, l, tick, c_next=False):
            h = hd(n)
            o = None
            tick()
            v_next = big[pl.ds(vrow(n), CK), :]
            if c_next:
                m_old = m_ref[...]
            l2 = None
            for j in range(NC):
                tick()
                vj = v_next
                if j + 1 < NC:
                    v_next = big[pl.ds(al(vrow(n) + (j + 1) * CK), CK), :]
                else:
                    w0 = big[pl.ds(worow(h), 256), :]
                oj = jnp.dot(big[prow(j), :], vj, preferred_element_type=F32)
                o = oj if o is None else o + oj
                if c_next:
                    pa = jnp.exp(s_ref[:, pl.ds(j * CK, 128)] - m_old)
                    pb = jnp.exp(s_ref[:, pl.ds(j * CK + 128, 128)] - m_old)
                    lj = pa + pb
                    l2 = lj if l2 is None else l2 + lj
                    big[prow(j), :] = jnp.concatenate([pa, pb], axis=1).astype(BF)
            o = (o / l).astype(BF)
            tick()
            w1 = big[pl.ds(al(worow(h) + 256), D - 256), :]
            y0 = lax.dot_general(o, w0, NT, preferred_element_type=F32)
            y1 = lax.dot_general(o, w1, NT, preferred_element_type=F32)
            b = bt(n)
            acc_ref[b, :, pl.ds(0, 256)] += y0
            acc_ref[b, :, pl.ds(256, D - 256)] += y1
            if c_next:
                return jnp.sum(l2, axis=-1, keepdims=True)

        def out_cast(b):
            o_buf[b] = acc_ref[b].astype(o_buf.dtype)

        notick = lambda: None
        i32 = jnp.int32
        x_cp(0).start(priority=0)
        wq_cp(0, 0, D).start(priority=1)
        k_part(i32(0), 0, Sk).start(priority=1)
        x_cp(1).start(priority=0)
        k_part(i32(1), 0, Sk).start(priority=1)
        wo_cp(0, 0, D).start(priority=1)
        v_cp(i32(0)).start(priority=1)
        v_cp(i32(1)).start(priority=1)
        acc_ref[...] = jnp.zeros_like(acc_ref)
        x_cp(0).wait()
        wq_cp(0, 0, D).wait()
        k_part(i32(0), 0, Sk).wait()
        stage_abc(i32(0), notick, True, False)

        def iteration(i, tb, ti):
            h = hd(i); b = bt(i)
            pos = [0]
            cnt = [0]
            def ktick(r):
                if r:
                    k_part(i + 2, pos[0], r).start(priority=0)
                    pos[0] += r
            wpred = jnp.logical_and(b < B - 1, h < H - 1)
            def issue_lo():
                @pl.when(wpred)
                def _():
                    wo_cp(h + 1, al(b * WS), WS).start(priority=1)
                v_cp(i + 2).start(priority=1)
            def tick():
                t = cnt[0]; cnt[0] += 1
                if t == lo_at:
                    issue_lo()
                if t == 0:
                    @pl.when(wpred)
                    def _():
                        wq_cp(h + 1, al(b * WS), WS).start(priority=0)
                    @pl.when(i + 2 < B)
                    def _():
                        x_cp(i + 2).start(priority=0)
                ktick(tb[t])
            for t, r in enumerate(ti):
                ktick(r)
                if t + 1 < len(ti):
                    pl.delay(DELAY)
            @pl.when(b == 0)
            def _():
                wo_cp(h, 0, D).wait()
            @pl.when(b == B - 1)
            def _():
                wq_cp(h + 1, 0, D).wait()
            @pl.when(i + 1 < B)
            def _():
                x_cp(i + 1).wait()
            k_part(i + 1, 0, Sk).wait()
            v_cp(i).wait()
            l = stage_abc(i + 1, tick, True, True)
            stage_de(i, l, tick)
            @pl.when(h == H - 1)
            def _():
                out_cast(b)
                if not defer:
                    o_cp(b, 1, b).start(priority=1)

        def body(i, c):
            if scopes:
                with jax.named_scope("it"):
                    iteration(i, TB, TI)
            else:
                iteration(i, TB, TI)
            return c
        lax.fori_loop(0, N - 3, body, 0)
        z = lax.fori_loop(0, 1, lambda t, c: c, i32(0)) if False else i32(0)
        iteration(i32(N - 3) + z, TL, [])
        if defer:
            o_cp(0, B - 2, 0).start(priority=1)
        k_part(i32(N - 1), 0, Sk).wait()
        l = stage_abc(i32(N - 1) + z, notick, True, True)
        v_cp(i32(N - 2)).wait()
        l = stage_de(i32(N - 2) + z, l, notick, c_next=True)
        out_cast(B - 2)
        o_cp(B - 2, 1, B - 2).start(priority=1)
        v_cp(i32(N - 1)).wait()
        stage_de(i32(N - 1) + z, l, notick)
        out_cast(B - 1)
        o_cp(B - 1, 1, B - 1).start(priority=0)
        if defer:
            o_cp(0, B - 2, 0).wait()
        else:
            for b in range(B - 2):
                o_cp(b, 1, b).wait()
        o_cp(B - 2, 1, B - 2).wait()
        o_cp(B - 1, 1, B - 1).wait()

    @jax.jit
    def f(x, kc, vc, wq, wo):
        B, Sq, D = x.shape
        _, H, Sk, Dh = kc.shape
        anyspec = pl.BlockSpec(memory_space=pl.ANY)
        return pl.pallas_call(
            kern,
            in_specs=[anyspec] * 5,
            out_specs=anyspec,
            out_shape=jax.ShapeDtypeStruct((B, Sq, D), x.dtype),
            scratch_shapes=[pltpu.VMEM((B, Sq, D), BF), pltpu.VMEM(((2 + NVB) * Sk + 4 * D + NC * Sq, Dh), BF),
                            pltpu.VMEM((Sq, Sk), F32), pltpu.VMEM((Sq, 128), F32),
                            pltpu.VMEM((B, Sq, D), F32), pltpu.VMEM((B, Sq, D), BF),
                            pltpu.SemaphoreType.DMA((2,)), pltpu.SemaphoreType.DMA((NVB,)),
                            pltpu.SemaphoreType.DMA((2,)),
                            pltpu.SemaphoreType.DMA((B,)), pltpu.SemaphoreType.DMA((B,))],
            compiler_params=pltpu.CompilerParams(vmem_limit_bytes=100 * 1024 * 1024, disable_bounds_checks=True),
        )(x, kc, vc, wq, wo.T)
    return f


_impl = make()


@jax.jit
def pallas_standalone__mha_block_cached__near_ridge_kernel(
    x: jax.Array,
    k_cache: jax.Array,
    v_cache: jax.Array,
    wq: jax.Array,
    wo: jax.Array,
):
    return _impl(x, k_cache, v_cache, wq, wo)
```

```python
import contextlib
import jax, jax.numpy as jnp
from jax import lax
from jax.experimental import pallas as pl
from jax.experimental.pallas import tpu as pltpu

NT = (((1,), (1,)), ((), ()))
F32 = jnp.float32
BF = jnp.bfloat16

def make(TX=None, TI=None, TY=None, NY2=12, DELAY=110, RL=None, scopes=False, lo_at=1, W1=2, PC=64, RG=16, NSP=0, nobc=True):
    maxin = 'y'
    TX = TX or [128,80,80,80,80,80,80,80,128]
    TI = TI if TI is not None else [80,80,112]
    TY = TY or [0,0,112,80,80,80,80,80,80,112, 64,0,0,80,0,0,0,112,0,0]
    NVB = 3
    NC = 8
    def kern(x_hbm, k_hbm, v_hbm, wq_hbm, wot_hbm, o_hbm,
             x_buf, wq_buf, wot_buf, big, s_ref, m_ref, l_ref, acc_ref, o_buf,
             ksem, vsem, wsem, osem):
        B, H, Sk, Dh = k_hbm.shape
        _, Sq, D = o_hbm.shape
        N = B * H
        CK = Sk // NC
        assert sum(TX) + sum(TI) + sum(TY) == Sk, sum(TX) + sum(TI) + sum(TY)
        assert len(TX) == 9 and len(TY) == 11 + Sq // RG
        KA = sum(TY[len(TY) - NY2:])
        NTAIL = (len(TI) - 1) if RL else 0
        VB = Sk - NTAIL * (RL or 0)
        K0 = 0
        V0 = 2 * Sk
        P0 = V0 + NVB * Sk
        def al(v):
            return pl.multiple_of(v, 64)
        def krow(n): return al(K0 + lax.rem(n, 2) * Sk)
        def vrow(n): return al(V0 + lax.rem(n, NVB) * Sk)
        hd = lambda n: lax.rem(n, H)
        bt = lambda n: lax.div(n, H)
        sc = (lambda nm: jax.named_scope(nm)) if scopes else (lambda nm: contextlib.nullcontext())

        def k_part(n, r0, cnt):
            return pltpu.make_async_copy(k_hbm.at[bt(n), hd(n), pl.ds(r0, cnt)],
                                         big.at[pl.ds(pl.multiple_of(krow(n) + r0, 16), cnt)], ksem.at[lax.rem(n, 2)])
        def v_part(n, r0, cnt):
            return pltpu.make_async_copy(v_hbm.at[bt(n), hd(n), pl.ds(r0, cnt)],
                                         big.at[pl.ds(pl.multiple_of(vrow(n) + r0, 16), cnt)], vsem.at[lax.rem(n, NVB)])
        def v_start(n):
            v_part(n, 0, VB).start(priority=1)
            for t in range(NTAIL):
                v_part(n, VB + t * RL, RL).start(priority=1)
        def o_cp(b0, cnt, s):
            return pltpu.make_async_copy(o_buf.at[pl.ds(b0, cnt)], o_hbm.at[pl.ds(b0, cnt)], osem.at[s])
        def prow(j):
            return pl.ds(P0 + j * Sq, Sq)
        def hcol(h, off, cnt):
            return pl.ds(pl.multiple_of(h * Dh + off, 128), cnt)

        def cgroup(g):
            rows = pl.ds(g * RG, RG)
            sg = s_ref[rows, :]
            m = jnp.max(sg, axis=-1, keepdims=True)
            p = jnp.exp(sg - m)
            l_ref[rows, :] = jnp.broadcast_to(1.0 / jnp.sum(p, axis=-1, keepdims=True), (RG, 128))
            pb = p.astype(BF)
            for j in range(NC):
                big[pl.ds(P0 + j * Sq + g * RG, RG), :] = pb[:, j * CK:(j + 1) * CK]

        def stage_x(n, tick):
            x = x_buf[pl.ds(pl.multiple_of(bt(n) * Sq, 16), Sq), :]
            q = jnp.dot(x, wq_buf[:, hcol(hd(n), 0, Dh)], preferred_element_type=F32)
            q = (q * (Dh ** -0.5)).astype(BF)
            m = None
            for j in range(NC):
                tick()
                kj = big[pl.ds(al(krow(n) + j * CK), CK), :]
                sj = lax.dot_general(q, kj, NT, preferred_element_type=F32)
                s_ref[:, pl.ds(j * CK, CK)] = sj
                if maxin == "x":
                    mj = jnp.maximum(sj[:, :128], sj[:, 128:])
                    m = mj if m is None else jnp.maximum(m, mj)
            tick()
            if maxin == "x":
                m_ref[...] = jnp.broadcast_to(jnp.max(m, axis=-1, keepdims=True), m_ref.shape)

        def stage_c(tick):
            for g in range(Sq // RG):
                cgroup(g)
                tick()

        def stage_y(n, tick, c_next):
            o = None
            tick()
            v_next = big[pl.ds(vrow(n), CK), :]
            for j in range(NC):
                tick()
                vj = v_next
                if j + 1 < NC:
                    v_next = big[pl.ds(al(vrow(n) + (j + 1) * CK), CK), :]
                oj = jnp.dot(big[prow(j), :], vj, preferred_element_type=F32)
                o = oj if o is None else o + oj
            tick()
            rl = l_ref[...]
            o = (o * jnp.concatenate([rl, rl], axis=1)).astype(BF)
            y = lax.dot_general(o, wot_buf[:, hcol(hd(n), 0, Dh)], NT, preferred_element_type=F32)
            acc_ref[...] += y
            if c_next:
                stage_c(tick)

        notick = lambda: None
        i32 = jnp.int32
        WC = PC * Dh // 8
        nwc = (H * Dh) // WC
        def w_chunk(src, dst, t, sem):
            r = pl.ds(pl.multiple_of(lax.div(t, nwc) * 8, 8), 8)
            c = pl.ds(pl.multiple_of(lax.rem(t, nwc) * WC, 128), WC)
            return pltpu.make_async_copy(src.at[r, c], dst.at[r, c], sem)
        XR = 32
        def x_chunk(t):
            r = pl.ds(pl.multiple_of(t * XR, XR), XR)
            return pltpu.make_async_copy(x_hbm.at[r], x_buf.at[r], wsem.at[2])
        def p1(t, c):
            w_chunk(wq_hbm, wq_buf, t, wsem.at[0]).start(priority=0)
            w_chunk(wot_hbm, wot_buf, t, wsem.at[1]).start(priority=1)
            return c
        lax.fori_loop(0, (D // 8) * nwc, p1, 0)
        acc_ref[...] = jnp.zeros_like(acc_ref)
        nk = Sk // PC
        nx = (B * Sq) // XR
        def p2(t, c):
            @pl.when(t < nk)
            def _():
                k_part(i32(0), pl.multiple_of(t * PC, PC), PC).start(priority=0)
            @pl.when(t < nx)
            def _():
                x_chunk(t).start(priority=1)
            return c
        lax.fori_loop(0, max(nk, nx), p2, 0)
        def p3(t, c):
            k_part(i32(1), pl.multiple_of(t * PC, PC), PC).start(priority=0)
            v_part(i32(0), pl.multiple_of(t * PC, PC), PC).start(priority=1)
            return c
        lax.fori_loop(0, nk, p3, 0)
        v_start(i32(1))
        pltpu.make_async_copy(wq_hbm, wq_buf, wsem.at[0]).wait()
        pltpu.make_async_copy(wot_hbm, wot_buf, wsem.at[1]).wait()
        pltpu.make_async_copy(x_hbm, x_buf, wsem.at[2]).wait()
        k_part(i32(0), 0, Sk).wait()
        stage_x(i32(0), notick)
        if KA:
            k_part(i32(2), 0, KA).start(priority=0)
        stage_c(notick)

        def iteration(i):
            rows = TX + TI + TY
            pos = [KA]
            cnt = [0]
            def tick():
                t = cnt[0]; cnt[0] += 1
                if t == lo_at:
                    v_start(i + 2)
                r = rows[t]
                if t == len(rows) - NY2:
                    assert pos[0] == Sk
                    pos[0] = 0
                if r:
                    p0 = pos[0]
                    if t < len(rows) - NY2:
                        k_part(i + 2, p0, r).start(priority=0)
                    else:
                        @pl.when(i + 3 < N)
                        def _():
                            k_part(i + 3, p0, r).start(priority=0)
                    pos[0] += r
            k_part(i + 1, 0, Sk).wait()
            stage_x(i + 1, tick)
            if RL:
                if TI: tick()
                v_part(i, 0, VB).wait()
                for t in range(NTAIL):
                    tick()
                    v_part(i, VB + t * RL, RL).wait()
            elif NSP:
                RI = TI[0]
                assert all(r == RI for r in TI)
                p0 = pos[0]
                def idle(t, c):
                    @pl.when(lax.rem(t, NSP) == 0)
                    def _():
                        k_part(i + 2, pl.multiple_of(p0 + lax.div(t, NSP) * RI, 16), RI).start(priority=0)
                    return c
                lax.fori_loop(0, (len(TI) - 1) * NSP + 1, idle, 0)
                pos[0] += RI * len(TI)
                cnt[0] += len(TI)
                v_part(i, 0, Sk).wait()
            else:
                for t in range(len(TI)):
                    pl.delay(DELAY if t else 1)
                    tick()
                v_part(i, 0, Sk).wait()
            stage_y(i, tick, True)
            @pl.when(hd(i) == H - 1)
            def _():
                o_buf[bt(i)] = acc_ref[...].astype(o_buf.dtype)
                acc_ref[...] = jnp.zeros_like(acc_ref)
            tick()

        def body(i, c):
            with sc("it"):
                iteration(i)
            return c
        lax.fori_loop(0, N - 2, body, 0)
        with sc("t1_waitK"):
            k_part(i32(N - 1), 0, Sk).wait()
        with sc("t2_X"):
            stage_x(i32(N - 1), notick)
        with sc("t3_waitV126"):
            v_part(i32(N - 2), 0, Sk).wait()
        if W1:
            o_cp(0, W1, 0).start(priority=1)
        with sc("t4_Y"):
            stage_y(i32(N - 2), notick, True)
        with sc("t5_waitV127"):
            v_part(i32(N - 1), 0, Sk).wait()
        o_cp(W1, B - 1 - W1, 1).start(priority=1)
        with sc("t6_Z"):
            stage_y(i32(N - 1), notick, False)
            o_buf[B - 1] = acc_ref[...].astype(o_buf.dtype)
            o_cp(B - 1, 1, 2).start(priority=0)
        with sc("t7_waitO"):
            if W1:
                o_cp(0, W1, 0).wait()
            o_cp(W1, B - 1 - W1, 1).wait()
        with sc("t8_waitOlast"):
            o_cp(B - 1, 1, 2).wait()

    @jax.jit
    def f(x, kc, vc, wq, wo):
        B, Sq, D = x.shape
        _, H, Sk, Dh = kc.shape
        anyspec = pl.BlockSpec(memory_space=pl.ANY)
        return pl.pallas_call(
            kern,
            in_specs=[anyspec] * 5,
            out_specs=anyspec,
            out_shape=jax.ShapeDtypeStruct((B, Sq, D), x.dtype),
            scratch_shapes=[pltpu.VMEM((B * Sq, D), BF), pltpu.VMEM((D, H * Dh), BF), pltpu.VMEM((D, H * Dh), BF),
                            pltpu.VMEM(((2 + NVB) * Sk + NC * Sq, Dh), BF),
                            pltpu.VMEM((Sq, Sk), F32), pltpu.VMEM((Sq, 128), F32), pltpu.VMEM((Sq, 128), F32),
                            pltpu.VMEM((Sq, D), F32), pltpu.VMEM((B, Sq, D), BF),
                            pltpu.SemaphoreType.DMA((2,)), pltpu.SemaphoreType.DMA((NVB,)),
                            pltpu.SemaphoreType.DMA((3,)), pltpu.SemaphoreType.DMA((3,))],
            compiler_params=pltpu.CompilerParams(vmem_limit_bytes=100 * 1024 * 1024, disable_bounds_checks=nobc),
        )(x.reshape(B * Sq, D), kc, vc, wq, wo.T)
    return f


_impl = make(W1=1, TX=[112,80,80,80,80,80,80,80,128], TI=[96,96,96], NSP=8)


@jax.jit
def pallas_standalone__mha_block_cached__near_ridge_kernel(
    x: jax.Array,
    k_cache: jax.Array,
    v_cache: jax.Array,
    wq: jax.Array,
    wo: jax.Array,
):
    return _impl(x, k_cache, v_cache, wq, wo)
```

```python
import contextlib
import jax, jax.numpy as jnp
from jax import lax
from jax.experimental import pallas as pl
from jax.experimental.pallas import tpu as pltpu

NT = (((1,), (1,)), ((), ()))
F32 = jnp.float32
BF = jnp.bfloat16

DEF = dict(
    x0=96, x0b=48, x1=80, x2=80, x3=80, x4=64, x5=80, x6=64, x7=80, x8=64, x9=112,
    y0=0, y1=0, y2=112, y3=80, y4=80, y5=80, y6=80, y7=80, y8=80, y9=64, yo=80,
    c0=64, c1=0, c2=0, c3=0, c4=64, c5=0, c6=0, c7=96, c8=0, e=0)

def make(T=None, RI=80, NI=3, NSP=8, ka="y8", scopes=False, lo_at="x1", W1=1, PC=64, RG=16, nobc=True,
         p1=True, p2=True, p3=False, p4=True, qwin=2, og=6, kf=32, VW={1: -1, 2: 0}):
    TT = dict(DEF); TT.update(T or {})
    NVB = 3
    NC = 8
    def kern(x_hbm, k_hbm, v_hbm, wq_hbm, wot_hbm, o_hbm,
             x_buf, wq_buf, wot_buf, big, s_ref, l_ref, acc_ref, o_buf,
             ksem, vsem, wsem, osem):
        B, H, Sk, Dh = k_hbm.shape
        _, Sq, D = o_hbm.shape
        N = B * H
        CK = Sk // NC
        names = list(TT)
        assert sum(TT.values()) + RI * NI == Sk, sum(TT.values()) + RI * NI
        KA = sum(TT[n] for n in names[names.index(ka):])
        K0 = 0
        V0 = 2 * Sk
        P0 = V0 + NVB * Sk
        Q0 = P0 + NC * Sq
        O0 = Q0 + 16
        def al(v):
            return pl.multiple_of(v, 64)
        def krow(n): return al(K0 + lax.rem(n, 2) * Sk)
        def vrow(n): return al(V0 + lax.rem(n, NVB) * Sk)
        hd = lambda n: lax.rem(n, H)
        bt = lambda n: lax.div(n, H)
        sc = (lambda nm: jax.named_scope(nm)) if scopes else (lambda nm: contextlib.nullcontext())

        def k_part(n, r0, cnt):
            return pltpu.make_async_copy(k_hbm.at[bt(n), hd(n), pl.ds(r0, cnt)],
                                         big.at[pl.ds(pl.multiple_of(krow(n) + r0, 16), cnt)], ksem.at[lax.rem(n, 2)])
        def v_part(n, r0, cnt):
            return pltpu.make_async_copy(v_hbm.at[bt(n), hd(n), pl.ds(r0, cnt)],
                                         big.at[pl.ds(pl.multiple_of(vrow(n) + r0, 16), cnt)], vsem.at[lax.rem(n, NVB)])
        def o_cp(b0, cnt, s):
            return pltpu.make_async_copy(o_buf.at[pl.ds(b0, cnt)], o_hbm.at[pl.ds(b0, cnt)], osem.at[s])
        def prow(j):
            return pl.ds(P0 + j * Sq, Sq)
        def hcol(h):
            return pl.ds(pl.multiple_of(h * Dh, Dh), Dh)

        def cgroup(g):
            rows = pl.ds(g * RG, RG)
            sg = s_ref[rows, :]
            m = jnp.max(sg, axis=-1, keepdims=True)
            p = jnp.exp(sg - m)
            l_ref[rows, :] = jnp.broadcast_to(1.0 / jnp.sum(p, axis=-1, keepdims=True), (RG, 128))
            pb = p.astype(BF)
            for j in range(NC):
                big[pl.ds(P0 + j * Sq + g * RG, RG), :] = pb[:, j * CK:(j + 1) * CK]

        def stage_x(n, tick, pins):
            x = x_buf[pl.ds(pl.multiple_of(bt(n) * Sq, 16), Sq), :]
            q = jnp.dot(x, wq_buf[:, hcol(hd(n))], preferred_element_type=F32)
            q = (q * (Dh ** -0.5)).astype(BF)
            for j in range(NC):
                tick(f"x{j}")
                if j == 0 and pins and p1:
                    ld = lambda r, c: big[pl.ds(pl.multiple_of(krow(n) + r, 16), c), :]
                    k1, k3 = ld(128 - kf, kf), ld(256 - kf, kf)
                    tick("x0b")
                    kj = jnp.concatenate([ld(0, 128 - kf), k1, ld(128, 128 - kf), k3], axis=0)
                else:
                    kj = big[pl.ds(al(krow(n) + j * CK), CK), :]
                qj = q
                if pins and p2:
                    if j == qwin:
                        big[pl.ds(Q0, 16), :] = q[Sq - 16:, :]
                    if j == NC - 1:
                        tick("x8")
                        qj = jnp.concatenate([q[:Sq - 16, :], big[pl.ds(Q0, 16), :]], axis=0)
                s_ref[:, pl.ds(j * CK, CK)] = lax.dot_general(qj, kj, NT, preferred_element_type=F32)
            tick("x9" if p2 else "x8")

        def stage_c(tick):
            for g in range(Sq // RG):
                cgroup(g)
                tick(f"c{g}")

        def stage_y(n, tick, c_next, pins):
            o = None
            vld = lambda j: big[pl.ds(al(vrow(n) + j * CK), CK), :]
            tick("y0")
            vwin = {j: j - 1 for j in range(NC)}
            if pins and p3:
                vwin.update(VW)
            vs = {j: vld(j) for j in range(NC) if vwin[j] < 0}
            for j in range(NC):
                tick(f"y{j + 1}")
                for jj in range(NC):
                    if vwin[jj] == j:
                        vs[jj] = vld(jj)
                pj = big[prow(j), :]
                oj = jnp.dot(pj, vs[j], preferred_element_type=F32)
                o = oj if o is None else o + oj
            tick("y9")
            rl = l_ref[...]
            o = (o * jnp.concatenate([rl, rl], axis=1)).astype(BF)
            if pins and p4:
                r0 = og * 16
                big[pl.ds(O0, 16), :] = o[r0:r0 + 16, :]
                tick("yo")
                parts = ([o[:r0]] if r0 else []) + [big[pl.ds(O0, 16), :]] + ([o[r0 + 16:]] if r0 + 16 < Sq else [])
                o1 = jnp.concatenate(parts, axis=0)
                y0 = lax.dot_general(o, wot_buf[pl.ds(0, 256), hcol(hd(n))], NT, preferred_element_type=F32)
                y1 = lax.dot_general(o1, wot_buf[pl.ds(256, D - 256), hcol(hd(n))], NT, preferred_element_type=F32)
                acc_ref[:, pl.ds(0, 256)] += y0
                acc_ref[:, pl.ds(256, D - 256)] += y1
            else:
                acc_ref[...] += lax.dot_general(o, wot_buf[:, hcol(hd(n))], NT, preferred_element_type=F32)
            if c_next:
                stage_c(tick)

        notick = lambda nm: None
        i32 = jnp.int32
        WC = PC * Dh // 8
        nwc = (H * Dh) // WC
        def w_chunk(src, dst, t, sem):
            r = pl.ds(pl.multiple_of(lax.div(t, nwc) * 8, 8), 8)
            c = pl.ds(pl.multiple_of(lax.rem(t, nwc) * WC, 128), WC)
            return pltpu.make_async_copy(src.at[r, c], dst.at[r, c], sem)
        XR = 32
        def x_chunk(t):
            r = pl.ds(pl.multiple_of(t * XR, XR), XR)
            return pltpu.make_async_copy(x_hbm.at[r], x_buf.at[r], wsem.at[2])
        def pr1(t, c):
            w_chunk(wq_hbm, wq_buf, t, wsem.at[0]).start(priority=0)
            w_chunk(wot_hbm, wot_buf, t, wsem.at[1]).start(priority=1)
            return c
        lax.fori_loop(0, (D // 8) * nwc, pr1, 0)
        acc_ref[...] = jnp.zeros_like(acc_ref)
        nk = Sk // PC
        nx = (B * Sq) // XR
        def pr2(t, c):
            @pl.when(t < nk)
            def _():
                k_part(i32(0), pl.multiple_of(t * PC, PC), PC).start(priority=0)
            @pl.when(t < nx)
            def _():
                x_chunk(t).start(priority=1)
            return c
        lax.fori_loop(0, max(nk, nx), pr2, 0)
        def pr3(t, c):
            k_part(i32(1), pl.multiple_of(t * PC, PC), PC).start(priority=0)
            v_part(i32(0), pl.multiple_of(t * PC, PC), PC).start(priority=1)
            return c
        lax.fori_loop(0, nk, pr3, 0)
        v_part(i32(1), 0, Sk).start(priority=1)
        pltpu.make_async_copy(wq_hbm, wq_buf, wsem.at[0]).wait()
        pltpu.make_async_copy(wot_hbm, wot_buf, wsem.at[1]).wait()
        pltpu.make_async_copy(x_hbm, x_buf, wsem.at[2]).wait()
        k_part(i32(0), 0, Sk).wait()
        stage_x(i32(0), notick, False)
        k_part(i32(2), 0, KA).start(priority=0)
        stage_c(notick)

        def iteration(i):
            pos = [KA]
            late = [False]
            used = []
            def tick(nm):
                used.append(nm)
                if nm == lo_at:
                    v_part(i + 2, 0, Sk).start(priority=1)
                r = TT[nm]
                if nm == ka:
                    assert pos[0] == Sk, pos[0]
                    pos[0] = 0
                    late[0] = True
                if r:
                    p0 = pos[0]
                    if not late[0]:
                        k_part(i + 2, p0, r).start(priority=0)
                    else:
                        @pl.when(i + 3 < N)
                        def _():
                            k_part(i + 3, p0, r).start(priority=0)
                    pos[0] += r
            k_part(i + 1, 0, Sk).wait()
            stage_x(i + 1, tick, True)
            p0 = pos[0]
            def idle(t, c):
                @pl.when(lax.rem(t, NSP) == 0)
                def _():
                    k_part(i + 2, pl.multiple_of(p0 + lax.div(t, NSP) * RI, 16), RI).start(priority=0)
                return c
            lax.fori_loop(0, (NI - 1) * NSP + 1, idle, 0)
            pos[0] += RI * NI
            v_part(i, 0, Sk).wait()
            stage_y(i, tick, True, True)
            @pl.when(hd(i) == H - 1)
            def _():
                o_buf[bt(i)] = acc_ref[...].astype(o_buf.dtype)
                acc_ref[...] = jnp.zeros_like(acc_ref)
            tick("e")
            assert pos[0] == KA and all(TT[n] == 0 for n in TT if n not in used), (pos[0], KA, used)

        def body(i, c):
            with sc("it"):
                iteration(i)
            return c
        lax.fori_loop(0, N - 2, body, 0)
        with sc("t1_waitK"):
            k_part(i32(N - 1), 0, Sk).wait()
        with sc("t2_X"):
            stage_x(i32(N - 1), notick, False)
        with sc("t3_waitV126"):
            v_part(i32(N - 2), 0, Sk).wait()
        if W1:
            o_cp(0, W1, 0).start(priority=1)
        with sc("t4_Y"):
            stage_y(i32(N - 2), notick, True, False)
        with sc("t5_waitV127"):
            v_part(i32(N - 1), 0, Sk).wait()
        o_cp(W1, B - 1 - W1, 1).start(priority=1)
        with sc("t6_Z"):
            stage_y(i32(N - 1), notick, False, False)
            o_buf[B - 1] = acc_ref[...].astype(o_buf.dtype)
            o_cp(B - 1, 1, 2).start(priority=0)
        with sc("t7_waitO"):
            if W1:
                o_cp(0, W1, 0).wait()
            o_cp(W1, B - 1 - W1, 1).wait()
        with sc("t8_waitOlast"):
            o_cp(B - 1, 1, 2).wait()

    @jax.jit
    def f(x, kc, vc, wq, wo):
        B, Sq, D = x.shape
        _, H, Sk, Dh = kc.shape
        anyspec = pl.BlockSpec(memory_space=pl.ANY)
        return pl.pallas_call(
            kern,
            in_specs=[anyspec] * 5,
            out_specs=anyspec,
            out_shape=jax.ShapeDtypeStruct((B, Sq, D), x.dtype),
            scratch_shapes=[pltpu.VMEM((B * Sq, D), BF), pltpu.VMEM((D, H * Dh), BF), pltpu.VMEM((D, H * Dh), BF),
                            pltpu.VMEM(((2 + NVB) * Sk + NC * Sq + 32, Dh), BF),
                            pltpu.VMEM((Sq, Sk), F32), pltpu.VMEM((Sq, 128), F32),
                            pltpu.VMEM((Sq, D), F32), pltpu.VMEM((B, Sq, D), BF),
                            pltpu.SemaphoreType.DMA((2,)), pltpu.SemaphoreType.DMA((NVB,)),
                            pltpu.SemaphoreType.DMA((3,)), pltpu.SemaphoreType.DMA((3,))],
            compiler_params=pltpu.CompilerParams(vmem_limit_bytes=100 * 1024 * 1024, disable_bounds_checks=nobc),
        )(x.reshape(B * Sq, D), kc, vc, wq, wo.T)
    return f


_impl = make()


@jax.jit
def pallas_standalone__mha_block_cached__near_ridge_kernel(
    x: jax.Array,
    k_cache: jax.Array,
    v_cache: jax.Array,
    wq: jax.Array,
    wo: jax.Array,
):
    return _impl(x, k_cache, v_cache, wq, wo)
```

```python
import functools
import contextlib
import jax, jax.numpy as jnp
from jax import lax
from jax.experimental import pallas as pl
from jax.experimental.pallas import tpu as pltpu

NT = (((1,), (1,)), ((), ()))
F32 = jnp.float32
BF = jnp.bfloat16

DEF = dict(
    x0=1, x0b=1, x1=1, x2=1, x3=1, x4=1, x5=1, x6=1, x7=1, x8=1, x9=2, i0=2,
    y0=0, y1=1, y2=2, y3=1, y4=1, y5=1, y6=2, y7=1, y8=2, y9=1, yo=2,
    c0=1, c1=0, c2=0, c3=1, c4=0, c5=1, c6=0, c7=1, c8=0, e=0)

def make(G=2, O1=48, O0=56, T=None, ka="y8", PHI=42, scopes=False, W1=1, RG=16, nobc=True,
         qwin=2, og=7, owin=5, kf=48, lomode="piece", tailp=2, wpin="y7", OL=56, NVB=4):
    TT = dict(DEF); TT.update(T or {})
    NC = 8
    NR = 4
    RR = 512
    PC = 64
    NS = 2 * G
    CPH = NC // G
    def kern(x_hbm, k_hbm, v_hbm, wq_hbm, wot_hbm, o_hbm,
             x_buf, wq_buf, wot_buf, big, q_ref, s_ref, m_ref, l_ref, op_ref, acc_ref, o_buf,
             ksem, vsem, wsem, osem):
        B, Sq, D = o_hbm.shape
        Dh = k_hbm.shape[-1]
        H = wq_hbm.shape[1] // Dh
        N = B * H
        Sk = NR * RR
        CK = Sk // NC
        W = Sk // G
        names = list(TT)
        NRND = RR // PC
        NP = NRND * NR
        assert sum(TT.values()) == NP, sum(TT.values())
        KA = sum(TT[n] for n in names[names.index(ka):])
        KP = 0
        VP = 2 * NR
        PP = VP + NVB * NR
        TP = PP + NC
        def kpl(n): return KP + lax.rem(n, 2) * NR
        def vpl(n): return VP + lax.rem(n, NVB) * NR
        grp = lambda n: lax.div(n, G)
        sub = lambda n: lax.rem(n, G)
        sc = (lambda nm: jax.named_scope(nm)) if scopes else (lambda nm: contextlib.nullcontext())

        def rnd_rows(r, off):
            lo = 0 if r == 0 else off + (r - 1) * PC
            hi = RR if r == NRND - 1 else off + r * PC
            return lo, hi - lo
        def kv_copy(src, dpl, sem, n, p0, np_, r0, cnt, c0=0, cc=None):
            srow = pl.multiple_of(sub(n) * RR + r0, 8)
            cols = pl.ds(c0, cc or Dh)
            return pltpu.make_async_copy(src.at[pl.ds(grp(n) * NR + p0, np_), pl.ds(srow, cnt), cols],
                                         big.at[pl.ds(dpl + p0, np_), pl.ds(r0, cnt), cols], sem)
        def k_cp(n, *a):
            return kv_copy(k_hbm, kpl(n), ksem.at[lax.rem(n, 2)], n, *a)
        def v_cp(n, *a):
            return kv_copy(v_hbm, vpl(n), vsem.at[lax.rem(n, NVB)], n, *a)
        def piece(cp, n, t, prio):
            r, p = t // NR, t % NR
            if O1 == O0:
                cp(n, p, 1, *rnd_rows(r, O0)).start(priority=prio)
            else:
                cp(n, p, 1, *rnd_rows(r, O1), 128, 128).start(priority=prio)
                cp(n, p, 1, *rnd_rows(r, O0), 0, 128).start(priority=prio)
        def v_rounds(n):
            for r in range(NRND):
                v_cp(n, 0, NR, *rnd_rows(r, OL)).start(priority=1)
        def o_cp(b0, cnt, s):
            return pltpu.make_async_copy(o_buf.at[pl.ds(b0, cnt)], o_hbm.at[pl.ds(b0, cnt)], osem.at[s])
        def hcol(h):
            return pl.ds(pl.multiple_of(h * Dh, Dh), Dh)
        def chunk(pl0, j, r0=0, cnt=None):
            return big[pl0 + j // 2, pl.ds((j % 2) * CK + r0, cnt or CK), :]

        def qproj(e):
            x = x_buf[pl.ds(pl.multiple_of(lax.div(e, H) * Sq, 16), Sq), :]
            q = jnp.dot(x, wq_buf[:, hcol(lax.rem(e, H))], preferred_element_type=F32)
            return (q * (Dh ** -0.5)).astype(BF)

        def stage_x(n, tick, pins, do_q=True):
            hs0 = lax.rem(grp(n) * G, NS)
            q = q_ref[hs0]
            if do_q:
                q_ref[lax.rem(n + G - 1, NS)] = qproj(jnp.minimum(n + G - 1, N - 1))
            for j in range(NC):
                if j and j % CPH == 0:
                    q = q_ref[hs0 + j // CPH]
                tick(f"x{j}")
                if j == 0 and pins:
                    k1, k3 = chunk(kpl(n), 0, 128 - kf, kf), chunk(kpl(n), 0, 256 - kf, kf)
                    tick("x0b")
                    kj = jnp.concatenate([chunk(kpl(n), 0, 0, 128 - kf), k1, chunk(kpl(n), 0, 128, 128 - kf), k3], axis=0)
                else:
                    kj = chunk(kpl(n), j)
                qj = q
                if pins:
                    if j == qwin:
                        big[TP, pl.ds(0, 16), :] = q_ref[hs0 + G - 1, pl.ds(Sq - 16, 16), :]
                    if j == NC - 1:
                        tick("x8")
                        qj = jnp.concatenate([q[:Sq - 16, :], big[TP, pl.ds(0, 16), :]], axis=0)
                s_ref[:, pl.ds(j * CK, CK)] = lax.dot_general(qj, kj, NT, preferred_element_type=F32)
            tick("x9")

        def stage_c(n, tick):
            hs0 = lax.rem(grp(n) * G, NS)
            u = sub(n)
            for g in range(Sq // RG):
                rows = pl.ds(g * RG, RG)
                for a in range(G):
                    sg = s_ref[rows, pl.ds(a * W, W)]
                    m = jnp.max(sg, axis=-1, keepdims=True)
                    p = jnp.exp(sg - m)
                    lp = p[:, :128]
                    for c in range(1, W // 128):
                        lp = lp + p[:, c * 128:(c + 1) * 128]
                    m_ref[hs0 + a, u, rows, :] = jnp.broadcast_to(m, (RG, 128))
                    l_ref[hs0 + a, u, rows, :] = lp
                    pb = p.astype(BF)
                    for jj in range(CPH):
                        big[PP + a * CPH + jj, rows, :] = pb[:, jj * CK:(jj + 1) * CK]
                tick(f"c{g}")

        def combine(e):
            hs = lax.rem(e + NS, NS)
            ms = [m_ref[hs, u] for u in range(G)]
            mx = functools.reduce(jnp.maximum, ms)
            al = [jnp.exp(m - mx) for m in ms]
            L = functools.reduce(lambda a, b: a + b, [al[u] * l_ref[hs, u] for u in range(G)])
            r = 1.0 / jnp.sum(L, axis=-1, keepdims=True)
            o = None
            for u in range(G):
                w = al[u] * r
                t = op_ref[hs, u] * jnp.concatenate([w, w], axis=1)
                o = t if o is None else o + t
            return o.astype(BF)

        def outproj(e, o0, o1=None):
            col = hcol(lax.rem(jnp.maximum(e, 0), H))
            if o1 is None:
                acc_ref[...] += lax.dot_general(o0, wot_buf[:, col], NT, preferred_element_type=F32)
            else:
                acc_ref[:, pl.ds(0, 256)] += lax.dot_general(o0, wot_buf[pl.ds(0, 256), col], NT, preferred_element_type=F32)
                acc_ref[:, pl.ds(256, D - 256)] += lax.dot_general(o1, wot_buf[pl.ds(256, D - 256), col], NT, preferred_element_type=F32)

        def stage_y(n, tick, c_next, pins):
            hs0 = lax.rem(grp(n) * G, NS)
            u = sub(n)
            e = n - (G - 1)
            tick("y0")
            v_next = chunk(vpl(n), 0)
            o = None
            for j in range(NC):
                tick(f"y{j + 1}")
                vj = v_next
                if j + 1 < NC:
                    v_next = chunk(vpl(n), j + 1)
                oj = jnp.dot(big[PP + j, pl.ds(0, Sq), :], vj, preferred_element_type=F32)
                o = oj if j % CPH == 0 else o + oj
                if j % CPH == CPH - 1:
                    op_ref[hs0 + j // CPH, u] = o
                if j == CPH - 1:
                    oc = combine(e)
                if pins and j == owin:
                    big[TP, pl.ds(16, 16), :] = oc[og * 16:og * 16 + 16, :]
            tick("y9")
            if pins:
                r0 = og * 16
                parts = ([oc[:r0]] if r0 else []) + [big[TP, pl.ds(16, 16), :]] + ([oc[r0 + 16:]] if r0 + 16 < Sq else [])
                o0 = jnp.concatenate(parts, axis=0)
                tick("yo")
                outproj(e, o0, oc)
            else:
                outproj(e, oc)
            if c_next:
                stage_c(n + 1, tick)

        notick = lambda nm: None
        i32 = jnp.int32
        WC = 64 * Dh // 8
        nwc = (H * Dh) // WC
        NW = (D // 8) * nwc
        def w_chunk(src, dst, t, sem):
            t = lax.rem(t, NR) * (NW // NR) + lax.div(t, NR)
            r = pl.ds(pl.multiple_of(lax.div(t, nwc) * 8, 8), 8)
            c = pl.ds(pl.multiple_of(lax.rem(t, nwc) * WC, 128), WC)
            return pltpu.make_async_copy(src.at[r, c], dst.at[r, c], sem)
        XR = 32
        nx = (B * Sq) // XR
        def x_chunk(t):
            t = lax.rem(t, 2) * (nx // 2) + lax.div(t, 2)
            r = pl.ds(pl.multiple_of(t * XR, XR), XR)
            return pltpu.make_async_copy(x_hbm.at[r], x_buf.at[r], wsem.at[2])
        def pr1(t, c):
            w_chunk(wq_hbm, wq_buf, t, wsem.at[0]).start(priority=0)
            w_chunk(wot_hbm, wot_buf, t, wsem.at[1]).start(priority=1)
            return c
        lax.fori_loop(0, 24, pr1, 0)
        acc_ref[...] = jnp.zeros_like(acc_ref)
        for hs in range(NS - G + 1, NS):
            op_ref[hs] = jnp.zeros(op_ref.shape[1:], F32)
            m_ref[hs] = jnp.zeros(m_ref.shape[1:], F32)
            l_ref[hs] = jnp.ones(l_ref.shape[1:], F32)
        lax.fori_loop(24, NW, pr1, 0)
        def dyn_piece(cp, n, t):
            return cp(n, lax.rem(t, NR), 1, pl.multiple_of(lax.div(t, NR) * PC, 8), PC)
        def pr2(t, c):
            @pl.when(t < NP)
            def _():
                dyn_piece(k_cp, i32(0), t).start(priority=0)
            @pl.when(t < nx)
            def _():
                x_chunk(t).start(priority=1)
            return c
        lax.fori_loop(0, max(NP, nx), pr2, 0)
        def pr3(t, c):
            dyn_piece(k_cp, i32(1), t).start(priority=0)
            dyn_piece(v_cp, i32(0), t).start(priority=1)
            return c
        lax.fori_loop(0, NP, pr3, 0)
        pltpu.make_async_copy(wq_hbm, wq_buf, wsem.at[0]).wait()
        pltpu.make_async_copy(wot_hbm, wot_buf, wsem.at[1]).wait()
        pltpu.make_async_copy(x_hbm, x_buf, wsem.at[2]).wait()
        k_cp(i32(0), 0, NR, 0, RR).wait()
        for e in range(G - 1):
            q_ref[e] = qproj(i32(e))
        assert PHI >= NP
        stage_x(i32(0), notick, False)
        if lomode == "piece":
            for t in range(PHI - NP):
                piece(v_cp, i32(1), t, 1)
        else:
            v_rounds(i32(1))
        for t in range(KA):
            piece(k_cp, i32(2), t, 0)
        stage_c(i32(0), notick)

        def iteration(i):
            cnt = [0]
            used = []
            def tick(nm):
                used.append(nm)
                for _ in range(TT[nm]):
                    t = cnt[0]; cnt[0] += 1
                    dk, tk = divmod(t + KA, NP)
                    if dk == 0:
                        piece(k_cp, i + 2, tk, 0)
                    else:
                        @pl.when(i + 3 < N)
                        def _():
                            piece(k_cp, i + 3, tk, 0)
                    if lomode == "piece":
                        dv, tv = divmod(t + PHI, NP)
                        piece(v_cp, i + dv, tv, 1)
            k_cp(i + 1, 0, NR, 0, RR).wait()
            stage_x(i + 1, tick, True)
            lax.fori_loop(0, jnp.minimum(i + 1, 1), lambda t, c: (tick("i0"), c)[1], 0)
            if lomode != "piece":
                v_rounds(i + 2)
            v_cp(i, 0, NR, 0, RR).wait()
            stage_y(i, tick, True, True)
            e = i - (G - 1)
            @pl.when(jnp.logical_and(e >= 0, lax.rem(e, H) == H - 1))
            def _():
                o_buf[lax.div(e, H)] = acc_ref[...].astype(o_buf.dtype)
                acc_ref[...] = jnp.zeros_like(acc_ref)
            tick("e")
            assert cnt[0] == NP and all(TT[n] == 0 for n in TT if n not in used), (cnt[0], used)

        def body(i, c):
            with sc("it"):
                iteration(i)
            return c
        lax.fori_loop(0, N - 2, body, 0)
        rest = list(range(PHI - NP, NP)) if lomode == "piece" else []
        def ttick(nm):
            for _ in range(tailp):
                for prio in (0, 1):
                    if rest:
                        piece(v_cp, i32(N - 1), rest.pop(0), prio)
        with sc("t1_waitK"):
            k_cp(i32(N - 1), 0, NR, 0, RR).wait()
        with sc("t2_X"):
            stage_x(i32(N - 1), ttick, False, do_q=False)
            assert not rest
        with sc("t3_waitV126"):
            v_cp(i32(N - 2), 0, NR, 0, RR).wait()
        with sc("t4_Y"):
            if W1:
                o_cp(0, W1, 0).start(priority=1)
            stage_y(i32(N - 2), notick, True, False)
        with sc("t5_waitV127"):
            v_cp(i32(N - 1), 0, NR, 0, RR).wait()
        o_cp(W1, B - 1 - W1, 1).start(priority=1)
        with sc("t6_Z"):
            stage_y(i32(N - 1), notick, False, False)
            for e in range(N - G + 1, N):
                outproj(i32(e), combine(i32(e)))
            o_buf[B - 1] = acc_ref[...].astype(o_buf.dtype)
            o_cp(B - 1, 1, 2).start(priority=0)
        with sc("t7_waitO"):
            if W1:
                o_cp(0, W1, 0).wait()
            o_cp(W1, B - 1 - W1, 1).wait()
        with sc("t8_waitOlast"):
            o_cp(B - 1, 1, 2).wait()

    @jax.jit
    def f(x, kc, vc, wq, wo):
        B, Sq, D = x.shape
        _, H, Sk, Dh = kc.shape
        anyspec = pl.BlockSpec(memory_space=pl.ANY)
        kvshape = (B * H * NR // G, RR * G, Dh)
        return pl.pallas_call(
            kern,
            in_specs=[anyspec] * 5,
            out_specs=anyspec,
            out_shape=jax.ShapeDtypeStruct((B, Sq, D), x.dtype),
            scratch_shapes=[pltpu.VMEM((B * Sq, D), BF), pltpu.VMEM((D, H * Dh), BF), pltpu.VMEM((D, H * Dh), BF),
                            pltpu.VMEM(((2 + NVB) * NR + NC + 1, RR, Dh), BF),
                            pltpu.VMEM((NS, Sq, Dh), BF),
                            pltpu.VMEM((Sq, Sk), F32),
                            pltpu.VMEM((NS, G, Sq, 128), F32), pltpu.VMEM((NS, G, Sq, 128), F32),
                            pltpu.VMEM((NS, G, Sq, Dh), F32),
                            pltpu.VMEM((Sq, D), F32), pltpu.VMEM((B, Sq, D), BF),
                            pltpu.SemaphoreType.DMA((2,)), pltpu.SemaphoreType.DMA((NVB,)),
                            pltpu.SemaphoreType.DMA((3,)), pltpu.SemaphoreType.DMA((3,))],
            compiler_params=pltpu.CompilerParams(vmem_limit_bytes=100 * 1024 * 1024, disable_bounds_checks=nobc),
        )(x.reshape(B * Sq, D), kc.reshape(kvshape), vc.reshape(kvshape), wq, wo.T)
    return f


_impl = make()


@jax.jit
def pallas_standalone__mha_block_cached__near_ridge_kernel(
    x: jax.Array,
    k_cache: jax.Array,
    v_cache: jax.Array,
    wq: jax.Array,
    wo: jax.Array,
):
    return _impl(x, k_cache, v_cache, wq, wo)
```

```python
import jax
import jax.numpy as jnp
from jax import lax
from jax.experimental import pallas as pl
from jax.experimental.pallas import tpu as pltpu

F32 = jnp.float32
BF16 = jnp.bfloat16
NT = (((1,), (1,)), ((), ()))

G = 2
NR = 4
RR = 512
PC = 64
NRND = RR // PC
NP = NRND * NR
NC = 8
CK = NR * RR // NC
CPH = NC // G
NS = 2 * G
NKB = 2
NVB = 4
RG = 16
OFF_HI, OFF_LO = 48, 56
TICKS = dict(x0=3, x1=1, x2=1, x3=1, x4=1, x5=1, x6=1, x7=1, x8=3,
             y1=2, y2=2, y3=1, y4=1, y5=1, y6=2, y7=1, y8=2, y9=2,
             c0=1, c1=1, c3=1, c5=1, c7=1)
KA = 10
VA = 10
PRO = 16
W1 = 6

KP = 0
VP = KP + NKB * NR
PP = VP + NVB * NR
NPLANES = PP + NC


def _kernel(x_hbm, k_hbm, v_hbm, wq_hbm, wot_hbm, o_hbm,
            x_buf, wq_buf, wot_buf, big, q_ref, s_ref, m_ref, l_ref, op_ref, acc_ref, o_buf,
            ksem, vsem, wsem, osem):
    B, Sq, D = o_hbm.shape
    Dh = k_hbm.shape[-1]
    H = wq_hbm.shape[1] // Dh
    N = B * H
    W = NR * RR // G
    i32 = jnp.int32
    assert sum(TICKS.values()) == NP

    def kpl(n):
        return KP + lax.rem(n, NKB) * NR

    def vpl(n):
        return VP + lax.rem(n, NVB) * NR

    def slot0(n):
        return lax.rem(lax.div(n, G) * G, NS)

    def kv_copy(src, dpl, sem, n, p0, np_, r0, cnt, c0=0, cc=None):
        srow = pl.multiple_of(lax.rem(n, G) * RR + r0, 8)
        cols = pl.ds(c0, cc or Dh)
        return pltpu.make_async_copy(
            src.at[pl.ds(lax.div(n, G) * NR + p0, np_), pl.ds(srow, cnt), cols],
            big.at[pl.ds(dpl + p0, np_), pl.ds(r0, cnt), cols], sem)

    def k_cp(n, *a):
        return kv_copy(k_hbm, kpl(n), ksem.at[lax.rem(n, NKB)], n, *a)

    def v_cp(n, *a):
        return kv_copy(v_hbm, vpl(n), vsem.at[lax.rem(n, NVB)], n, *a)

    def rows_of(r, off):
        lo = 0 if r == 0 else off + (r - 1) * PC
        hi = RR if r == NRND - 1 else off + r * PC
        return lo, hi - lo

    def piece(cp, n, t, prio):
        r, p = divmod(t, NR)
        cp(n, p, 1, *rows_of(r, OFF_HI), 128, 128).start(priority=prio)
        cp(n, p, 1, *rows_of(r, OFF_LO), 0, 128).start(priority=prio)

    def wait_slot(cp, n):
        cp(n, 0, NR, 0, RR).wait()

    def o_cp(b0, cnt, s):
        return pltpu.make_async_copy(o_buf.at[pl.ds(b0, cnt)], o_hbm.at[pl.ds(b0, cnt)], osem.at[s])

    def hcol(e):
        return pl.ds(pl.multiple_of(lax.rem(e, H) * Dh, Dh), Dh)

    def chunk(pl0, j):
        return big[pl0 + j // 2, pl.ds((j % 2) * CK, CK), :]

    def qproj(e):
        x = x_buf[pl.ds(pl.multiple_of(lax.div(e, H) * Sq, 16), Sq), :]
        q = jnp.dot(x, wq_buf[:, hcol(e)], preferred_element_type=F32)
        q_ref[lax.rem(e, NS)] = (q * (Dh ** -0.5)).astype(BF16)

    def stage_x(n, tick, with_q=True):
        hs0 = slot0(n)
        q = q_ref[hs0]
        if with_q:
            qproj(n + G - 1)
        for j in range(NC):
            if j and j % CPH == 0:
                q = q_ref[hs0 + j // CPH]
            tick(f"x{j}")
            s_ref[:, pl.ds(j * CK, CK)] = lax.dot_general(
                q, chunk(kpl(n), j), NT, preferred_element_type=F32)
        tick("x8")

    def stage_c(n, tick):
        hs0 = slot0(n)
        u = lax.rem(n, G)
        for g in range(Sq // RG):
            rows = pl.ds(g * RG, RG)
            for a in range(G):
                s = s_ref[rows, pl.ds(a * W, W)]
                m = jnp.max(s, axis=-1, keepdims=True)
                p = jnp.exp(s - m)
                lp = p[:, :128]
                for c in range(1, W // 128):
                    lp = lp + p[:, c * 128:(c + 1) * 128]
                m_ref[hs0 + a, u, rows, :] = jnp.broadcast_to(m, (RG, 128))
                l_ref[hs0 + a, u, rows, :] = lp
                pb = p.astype(BF16)
                for jj in range(CPH):
                    big[PP + a * CPH + jj, rows, :] = pb[:, jj * CK:(jj + 1) * CK]
            tick(f"c{g}")

    def merge(e):
        hs = lax.rem(e + NS, NS)
        m0, m1 = m_ref[hs, 0], m_ref[hs, 1]
        mx = jnp.maximum(m0, m1)
        a0, a1 = jnp.exp(m0 - mx), jnp.exp(m1 - mx)
        r = 1.0 / jnp.sum(a0 * l_ref[hs, 0] + a1 * l_ref[hs, 1], axis=-1, keepdims=True)
        w0, w1 = a0 * r, a1 * r
        o = (op_ref[hs, 0] * jnp.concatenate([w0, w0], axis=1)
             + op_ref[hs, 1] * jnp.concatenate([w1, w1], axis=1))
        return o.astype(BF16)

    def outproj(e, o):
        acc_ref[...] += lax.dot_general(
            o, wot_buf[:, hcol(jnp.maximum(e, 0))], NT, preferred_element_type=F32)

    def stage_y(n, tick):
        hs0 = slot0(n)
        u = lax.rem(n, G)
        v_next = chunk(vpl(n), 0)
        for j in range(NC):
            tick(f"y{j + 1}")
            vj = v_next
            if j + 1 < NC:
                v_next = chunk(vpl(n), j + 1)
            oj = jnp.dot(big[PP + j, pl.ds(0, Sq), :], vj, preferred_element_type=F32)
            o = oj if j % CPH == 0 else o + oj
            if j % CPH == CPH - 1:
                op_ref[hs0 + j // CPH, u] = o
            if j == CPH - 1:
                merged = merge(n - 1)
        tick("y9")
        outproj(n - 1, merged)

    WC = PC * Dh // 8
    nwc = (H * Dh) // WC
    NW = (D // 8) * nwc
    XR = 32
    NX = (B * Sq) // XR

    def w_piece(src, dst, t, sem):
        t = lax.rem(t, NR) * (NW // NR) + lax.div(t, NR)
        r = pl.ds(pl.multiple_of(lax.div(t, nwc) * 8, 8), 8)
        c = pl.ds(pl.multiple_of(lax.rem(t, nwc) * WC, 128), WC)
        return pltpu.make_async_copy(src.at[r, c], dst.at[r, c], sem)

    def x_piece(t):
        t = lax.rem(t, 2) * (NX // 2) + lax.div(t, 2)
        r = pl.ds(pl.multiple_of(t * XR, XR), XR)
        return pltpu.make_async_copy(x_hbm.at[r], x_buf.at[r], wsem.at[2])

    def plain_piece(cp, n, t):
        return cp(n, lax.rem(t, NR), 1, pl.multiple_of(lax.div(t, NR) * PC, 8), PC)

    def load_k0_x(t, c):
        plain_piece(k_cp, i32(0), t).start(priority=0)
        x_piece(t).start(priority=1)
        return c

    def load_x(t, c):
        x_piece(t).start(priority=1)
        return c

    def load_w(t, c):
        w_piece(wq_hbm, wq_buf, t, wsem.at[0]).start(priority=0)
        w_piece(wot_hbm, wot_buf, t, wsem.at[1]).start(priority=1)
        return c

    def load_k1_v0(t, c):
        plain_piece(k_cp, i32(1), t).start(priority=0)
        plain_piece(v_cp, i32(0), t).start(priority=1)
        return c

    lax.fori_loop(0, 24, load_k0_x, 0)
    acc_ref[...] = jnp.zeros_like(acc_ref)
    op_ref[NS - 1] = jnp.zeros(op_ref.shape[1:], F32)
    m_ref[NS - 1] = jnp.zeros(m_ref.shape[1:], F32)
    l_ref[NS - 1] = jnp.ones(l_ref.shape[1:], F32)
    lax.fori_loop(24, NP, load_k0_x, 0)
    lax.fori_loop(NP, NX, load_x, 0)
    lax.fori_loop(0, NW, load_w, 0)
    lax.fori_loop(0, NP - PRO, load_k1_v0, 0)
    pltpu.make_async_copy(wq_hbm, wq_buf, wsem.at[0]).wait()
    pltpu.make_async_copy(x_hbm, x_buf, wsem.at[2]).wait()
    wait_slot(k_cp, i32(0))

    todo = list(range(NP - PRO, NP))

    def pro_tick_x(name):
        for _ in range(2):
            if todo:
                load_k1_v0(i32(todo.pop(0)), 0)

    qproj(i32(0))
    stage_x(i32(0), pro_tick_x)
    assert not todo and KA == VA
    todo = list(range(KA))

    def pro_tick_c(name):
        if todo:
            t = todo.pop(0)
            piece(k_cp, i32(2), t, 0)
            piece(v_cp, i32(1), t, 1)

    pro_tick_c("pre")
    stage_c(i32(0), pro_tick_c)
    assert not todo
    pltpu.make_async_copy(wot_hbm, wot_buf, wsem.at[1]).wait()

    def iteration(i, carry):
        started = [0]

        def tick(name):
            for _ in range(TICKS.get(name, 0)):
                t = started[0]
                started[0] += 1
                dk, tk = divmod(t + KA, NP)
                if dk == 0:
                    piece(k_cp, i + 2, tk, 0)
                else:
                    @pl.when(i + 3 < N)
                    def _():
                        piece(k_cp, i + 3, tk, 0)
                dv, tv = divmod(t + VA, NP)
                piece(v_cp, i + 1 + dv, tv, 1)

        wait_slot(k_cp, i + 1)
        stage_x(i + 1, tick)
        wait_slot(v_cp, i)
        stage_y(i, tick)
        stage_c(i + 1, tick)
        assert started[0] == NP

        @pl.when(jnp.logical_and(i > 0, lax.rem(i, H) == 0))
        def _():
            o_buf[lax.div(i, H) - 1] = acc_ref[...].astype(o_buf.dtype)
            acc_ref[...] = jnp.zeros_like(acc_ref)

        return carry

    lax.fori_loop(0, N - 2, iteration, 0)

    todo = list(range(VA, NP))

    def tail_tick_x(name):
        for prio in (0, 1, 0, 1):
            if todo:
                piece(v_cp, i32(N - 1), todo.pop(0), prio)

    def tail_tick_y(name):
        if name == "y9":
            o_buf[B - 1, pl.ds(0, RG), pl.ds(0, Dh)] = (
                op_ref[(N - 1) % NS, 0, pl.ds(0, RG), :].astype(o_buf.dtype))
            o_cp(0, W1, 0).start(priority=1)

    def no_tick(name):
        pass

    wait_slot(k_cp, i32(N - 1))
    stage_x(i32(N - 1), tail_tick_x, with_q=False)
    assert not todo
    wait_slot(v_cp, i32(N - 2))
    stage_y(i32(N - 2), tail_tick_y)
    stage_c(i32(N - 1), no_tick)
    wait_slot(v_cp, i32(N - 1))
    o_cp(W1, B - 1 - W1, 1).start(priority=1)
    stage_y(i32(N - 1), no_tick)
    outproj(i32(N - 1), merge(i32(N - 1)))
    o_buf[B - 1] = acc_ref[...].astype(o_buf.dtype)
    o_cp(B - 1, 1, 2).start(priority=0)
    o_cp(0, W1, 0).wait()
    o_cp(W1, B - 1 - W1, 1).wait()
    o_cp(B - 1, 1, 2).wait()


@jax.jit
def pallas_standalone__mha_block_cached__near_ridge_kernel(
    x: jax.Array,
    k_cache: jax.Array,
    v_cache: jax.Array,
    wq: jax.Array,
    wo: jax.Array,
):
    B, Sq, D = x.shape
    _, H, Sk, Dh = k_cache.shape
    assert Sk == NR * RR and Dh == 256 and H % G == 0 and Sq % RG == 0
    in_hbm = pl.BlockSpec(memory_space=pl.ANY)
    kv_shape = (B * H * NR // G, RR * G, Dh)
    return pl.pallas_call(
        _kernel,
        in_specs=[in_hbm] * 5,
        out_specs=in_hbm,
        out_shape=jax.ShapeDtypeStruct((B, Sq, D), x.dtype),
        scratch_shapes=[
            pltpu.VMEM((B * Sq, D), BF16),
            pltpu.VMEM((D, H * Dh), BF16),
            pltpu.VMEM((D, H * Dh), BF16),
            pltpu.VMEM((NPLANES, RR, Dh), BF16),
            pltpu.VMEM((NS, Sq, Dh), BF16),
            pltpu.VMEM((Sq, Sk), F32),
            pltpu.VMEM((NS, G, Sq, 128), F32),
            pltpu.VMEM((NS, G, Sq, 128), F32),
            pltpu.VMEM((NS, G, Sq, Dh), F32),
            pltpu.VMEM((Sq, D), F32),
            pltpu.VMEM((B, Sq, D), BF16),
            pltpu.SemaphoreType.DMA((NKB,)),
            pltpu.SemaphoreType.DMA((NVB,)),
            pltpu.SemaphoreType.DMA((3,)),
            pltpu.SemaphoreType.DMA((3,)),
        ],
        compiler_params=pltpu.CompilerParams(
            vmem_limit_bytes=64 * 1024 * 1024, disable_bounds_checks=True),
    )(x.reshape(B * Sq, D), k_cache.reshape(kv_shape), v_cache.reshape(kv_shape), wq, wo.T)
```

```python
import jax
import jax.numpy as jnp
from jax import lax
from jax.experimental import pallas as pl
from jax.experimental.pallas import tpu as pltpu

F32 = jnp.float32
BF16 = jnp.bfloat16
NT = (((1,), (1,)), ((), ()))

G = 2
NR = 4
RR = 512
PC = 64
NRND = RR // PC
NP = NRND * NR
NC = 8
CK = NR * RR // NC
CPH = NC // G
NS = 2 * G
NKB = 2
NVB = 4
RG = 16
OFF_HI, OFF_LO = 48, 56
TICKS = dict(x0=3, x1=1, x2=1, x3=1, x4=1, x5=1, x6=1, x7=1, x8=3,
             y1=2, y2=2, y3=1, y4=1, y5=1, y6=2, y7=1, y8=2, y9=2,
             c0=1, c1=1, c3=1, c5=1, c7=1)
KA = 10
VA = 10
PRO = 16
W1 = 6

KP = 0
VP = KP + NKB * NR
PP = VP + NVB * NR
NPLANES = PP + NC


def _kernel(x_hbm, k_hbm, v_hbm, wq_hbm, wot_hbm, o_hbm,
            x_buf, wq_buf, wot_buf, big, q_ref, s_ref, m_ref, l_ref, op_ref, acc_ref, o_buf,
            ksem, vsem, wsem, osem):
    B, Sq, D = o_hbm.shape
    Dh = k_hbm.shape[-1]
    H = wq_hbm.shape[1] // Dh
    N = B * H
    W = NR * RR // G
    i32 = jnp.int32
    assert sum(TICKS.values()) == NP

    def kpl(n):
        return KP + lax.rem(n, NKB) * NR

    def vpl(n):
        return VP + lax.rem(n, NVB) * NR

    def slot0(n):
        return lax.rem(lax.div(n, G) * G, NS)

    def kv_copy(src, dpl, sem, n, p0, np_, r0, cnt, c0=0, cc=None):
        srow = pl.multiple_of(lax.rem(n, G) * RR + r0, 8)
        cols = pl.ds(c0, cc or Dh)
        return pltpu.make_async_copy(
            src.at[pl.ds(lax.div(n, G) * NR + p0, np_), pl.ds(srow, cnt), cols],
            big.at[pl.ds(dpl + p0, np_), pl.ds(r0, cnt), cols], sem)

    def k_cp(n, *a):
        return kv_copy(k_hbm, kpl(n), ksem.at[lax.rem(n, NKB)], n, *a)

    def v_cp(n, *a):
        return kv_copy(v_hbm, vpl(n), vsem.at[lax.rem(n, NVB)], n, *a)

    def rows_of(r, off):
        lo = 0 if r == 0 else off + (r - 1) * PC
        hi = RR if r == NRND - 1 else off + r * PC
        return lo, hi - lo

    def piece(cp, n, t, prio):
        r, p = divmod(t, NR)
        cp(n, p, 1, *rows_of(r, OFF_HI), 128, 128).start(priority=prio)
        cp(n, p, 1, *rows_of(r, OFF_LO), 0, 128).start(priority=prio)

    def wait_slot(cp, n):
        cp(n, 0, NR, 0, RR).wait()

    def o_cp(b0, cnt, s):
        return pltpu.make_async_copy(o_buf.at[pl.ds(b0, cnt)], o_hbm.at[pl.ds(b0, cnt)], osem.at[s])

    def hcol(e):
        return pl.ds(pl.multiple_of(lax.rem(e, H) * Dh, Dh), Dh)

    def chunk(pl0, j):
        return big[pl0 + j // 2, pl.ds((j % 2) * CK, CK), :]

    def qproj(e):
        x = x_buf[pl.ds(pl.multiple_of(lax.div(e, H) * Sq, 16), Sq), :]
        q = jnp.dot(x, wq_buf[:, hcol(e)], preferred_element_type=F32)
        q_ref[lax.rem(e, NS)] = (q * (Dh ** -0.5)).astype(BF16)

    def stage_x(n, tick, with_q=True):
        hs0 = slot0(n)
        q = q_ref[hs0]
        if with_q:
            qproj(n + G - 1)
        for j in range(NC):
            if j and j % CPH == 0:
                q = q_ref[hs0 + j // CPH]
            tick(f"x{j}")
            s_ref[:, pl.ds(j * CK, CK)] = lax.dot_general(
                q, chunk(kpl(n), j), NT, preferred_element_type=F32)
        tick("x8")

    def c_group(n, g, pp, heads=range(G)):
        hs0 = slot0(n)
        u = lax.rem(n, G)
        rows = pl.ds(g * RG, RG)
        for a in heads:
            s = s_ref[rows, pl.ds(a * W, W)]
            m = jnp.max(s, axis=-1, keepdims=True)
            p = jnp.exp(s - m)
            lp = p[:, :128]
            for c in range(1, W // 128):
                lp = lp + p[:, c * 128:(c + 1) * 128]
            m_ref[hs0 + a, u, rows, :] = jnp.broadcast_to(m, (RG, 128))
            l_ref[hs0 + a, u, rows, :] = lp
            pb = p.astype(BF16)
            for jj in range(CPH):
                big[pp + a * CPH + jj, rows, :] = pb[:, jj * CK:(jj + 1) * CK]

    def stage_c(n, tick):
        for g in range(Sq // RG):
            c_group(n, g, PP)
            tick(f"c{g}")

    def merge(e):
        hs = lax.rem(e + NS, NS)
        m0, m1 = m_ref[hs, 0], m_ref[hs, 1]
        mx = jnp.maximum(m0, m1)
        a0, a1 = jnp.exp(m0 - mx), jnp.exp(m1 - mx)
        r = 1.0 / jnp.sum(a0 * l_ref[hs, 0] + a1 * l_ref[hs, 1], axis=-1, keepdims=True)
        w0, w1 = a0 * r, a1 * r
        o = (op_ref[hs, 0] * jnp.concatenate([w0, w0], axis=1)
             + op_ref[hs, 1] * jnp.concatenate([w1, w1], axis=1))
        return o.astype(BF16)

    def outproj(e, o):
        acc_ref[...] += lax.dot_general(
            o, wot_buf[:, hcol(jnp.maximum(e, 0))], NT, preferred_element_type=F32)

    def stage_y(n, tick, pp=PP):
        hs0 = slot0(n)
        u = lax.rem(n, G)
        v_next = chunk(vpl(n), 0)
        for j in range(NC):
            tick(f"y{j + 1}")
            vj = v_next
            if j + 1 < NC:
                v_next = chunk(vpl(n), j + 1)
            oj = jnp.dot(big[pp + j, pl.ds(0, Sq), :], vj, preferred_element_type=F32)
            o = oj if j % CPH == 0 else o + oj
            if j % CPH == CPH - 1:
                op_ref[hs0 + j // CPH, u] = o
            if j == CPH - 1:
                merged = merge(n - 1)
        tick("y9")
        outproj(n - 1, merged)

    XR = 32
    NX = (B * Sq) // XR

    def x_piece(t):
        t = lax.rem(t, 2) * (NX // 2) + lax.div(t, 2)
        r = pl.ds(pl.multiple_of(t * XR, XR), XR)
        return pltpu.make_async_copy(x_hbm.at[r], x_buf.at[r], wsem.at[2])

    def plain_piece(cp, n, t):
        return cp(n, lax.rem(t, NR), 1, pl.multiple_of(lax.div(t, NR) * PC, 8), PC)

    def load_k0_x(t, c):
        plain_piece(k_cp, i32(0), t).start(priority=0)
        x_piece(t).start(priority=1)
        return c

    def load_x(t, c):
        x_piece(t).start(priority=1)
        return c

    def load_w(t, c):
        nrow = D // 8
        def cp(src, dst, sem, row, c0, c1):
            r = pl.ds(pl.multiple_of(row * 8, 8), 8)
            cols = pl.ds(c0 * 128, (c1 - c0) * 128)
            return pltpu.make_async_copy(src.at[r, cols], dst.at[r, cols], sem)
        both = ((wq_hbm, wq_buf, wsem.at[0], 0), (wot_hbm, wot_buf, wsem.at[1], 1))
        for p in range(NR):
            for src, dst, sem, prio in both:
                cp(src, dst, sem, p * (nrow // NR) + t, 13, 29).start(priority=prio)
        for p in range(NR):
            row = p * (nrow // NR) + t
            nxt = jnp.where(row + 1 == nrow, 0, row + 1)
            for src, dst, sem, prio in both:
                cp(src, dst, sem, row, 29, 32).start(priority=prio)
                cp(src, dst, sem, nxt, 0, 13).start(priority=prio)
        return c

    def load_k1_v0(t, c):
        plain_piece(k_cp, i32(1), t).start(priority=0)
        plain_piece(v_cp, i32(0), t).start(priority=1)
        return c

    lax.fori_loop(0, 24, load_k0_x, 0)
    acc_ref[...] = jnp.zeros_like(acc_ref)
    op_ref[NS - 1] = jnp.zeros(op_ref.shape[1:], F32)
    m_ref[NS - 1] = jnp.zeros(m_ref.shape[1:], F32)
    l_ref[NS - 1] = jnp.ones(l_ref.shape[1:], F32)
    lax.fori_loop(24, NP, load_k0_x, 0)
    lax.fori_loop(NP, NX, load_x, 0)
    lax.fori_loop(0, D // 8 // NR, load_w, 0)
    lax.fori_loop(0, NP - PRO, load_k1_v0, 0)
    pltpu.make_async_copy(wq_hbm, wq_buf, wsem.at[0]).wait()
    pltpu.make_async_copy(x_hbm, x_buf, wsem.at[2]).wait()
    wait_slot(k_cp, i32(0))

    todo = list(range(NP - PRO, NP))

    def pro_tick_x(name):
        for _ in range(2):
            if todo:
                load_k1_v0(i32(todo.pop(0)), 0)

    qproj(i32(0))
    stage_x(i32(0), pro_tick_x)
    assert not todo
    todo = list(range(max(KA, VA)))

    def pro_tick_c(name):
        for _ in range(2):
            if todo:
                t = todo.pop(0)
                if t < KA:
                    piece(k_cp, i32(2), t, 0)
                if t < VA:
                    piece(v_cp, i32(1), t, 1)

    pro_tick_c("pre")
    stage_c(i32(0), pro_tick_c)
    assert not todo
    pltpu.make_async_copy(wot_hbm, wot_buf, wsem.at[1]).wait()

    def iteration(i, carry):
        started = [0]

        def tick(name):
            for _ in range(TICKS.get(name, 0)):
                t = started[0]
                started[0] += 1
                dk, tk = divmod(t + KA, NP)
                if dk == 0:
                    piece(k_cp, i + 2, tk, 0)
                else:
                    @pl.when(i + 3 < N)
                    def _():
                        piece(k_cp, i + 3, tk, 0)
                dv, tv = divmod(t + VA, NP)
                piece(v_cp, i + 1 + dv, tv, 1)

        wait_slot(k_cp, i + 1)
        stage_x(i + 1, tick)
        wait_slot(v_cp, i)
        stage_y(i, tick)
        stage_c(i + 1, tick)
        assert started[0] == NP

        @pl.when(jnp.logical_and(i > 0, lax.rem(i, H) == 0))
        def _():
            o_buf[lax.div(i, H) - 1] = acc_ref[...].astype(o_buf.dtype)
            acc_ref[...] = jnp.zeros_like(acc_ref)

        return carry

    lax.fori_loop(0, N - 2, iteration, 0)

    todo = list(range(VA, NP))

    def tail_tick_x(name):
        for prio in (0, 1, 0, 1):
            if todo:
                piece(v_cp, i32(N - 1), todo.pop(0), prio)

    def tail_tick_y(name):
        if name == "y9":
            o_buf[B - 1, pl.ds(0, RG), pl.ds(0, Dh)] = (
                op_ref[(N - 1) % NS, 0, pl.ds(0, RG), :].astype(o_buf.dtype))
            o_cp(0, W1, 0).start(priority=1)

    def no_tick(name):
        pass

    wait_slot(k_cp, i32(N - 1))
    stage_x(i32(N - 1), tail_tick_x, with_q=False)
    assert not todo
    for g in range(Sq // RG):
        c_group(i32(N - 1), g, KP, [0])
    wait_slot(v_cp, i32(N - 2))
    stage_y(i32(N - 2), tail_tick_y)
    for g in range(Sq // RG):
        c_group(i32(N - 1), g, KP, [1])
    wait_slot(v_cp, i32(N - 1))
    o_cp(W1, B - 1 - W1, 1).start(priority=1)
    stage_y(i32(N - 1), no_tick, KP)
    o = merge(i32(N - 1))
    last = []
    for k, (c0, cc) in enumerate(((0, 256), (256, D - 256))):
        cols = pl.ds(c0, cc)
        y = lax.dot_general(o, wot_buf[cols, hcol(i32(N - 1))], NT, preferred_element_type=F32)
        o_buf[B - 1, :, cols] = (acc_ref[:, cols] + y).astype(o_buf.dtype)
        last.append(pltpu.make_async_copy(o_buf.at[B - 1, :, cols], o_hbm.at[B - 1, :, cols], osem.at[2 + k]))
        last[-1].start(priority=0)
    o_cp(0, W1, 0).wait()
    o_cp(W1, B - 1 - W1, 1).wait()
    for c in last:
        c.wait()


@jax.jit
def pallas_standalone__mha_block_cached__near_ridge_kernel(
    x: jax.Array,
    k_cache: jax.Array,
    v_cache: jax.Array,
    wq: jax.Array,
    wo: jax.Array,
):
    B, Sq, D = x.shape
    _, H, Sk, Dh = k_cache.shape
    assert Sk == NR * RR and Dh == 256 and H % G == 0 and Sq % RG == 0
    in_hbm = pl.BlockSpec(memory_space=pl.ANY)
    kv_shape = (B * H * NR // G, RR * G, Dh)
    return pl.pallas_call(
        _kernel,
        in_specs=[in_hbm] * 5,
        out_specs=in_hbm,
        out_shape=jax.ShapeDtypeStruct((B, Sq, D), x.dtype),
        scratch_shapes=[
            pltpu.VMEM((B * Sq, D), BF16),
            pltpu.VMEM((D, H * Dh), BF16),
            pltpu.VMEM((D, H * Dh), BF16),
            pltpu.VMEM((NPLANES, RR, Dh), BF16),
            pltpu.VMEM((NS, Sq, Dh), BF16),
            pltpu.VMEM((Sq, Sk), F32),
            pltpu.VMEM((NS, G, Sq, 128), F32),
            pltpu.VMEM((NS, G, Sq, 128), F32),
            pltpu.VMEM((NS, G, Sq, Dh), F32),
            pltpu.VMEM((Sq, D), F32),
            pltpu.VMEM((B, Sq, D), BF16),
            pltpu.SemaphoreType.DMA((NKB,)),
            pltpu.SemaphoreType.DMA((NVB,)),
            pltpu.SemaphoreType.DMA((3,)),
            pltpu.SemaphoreType.DMA((4,)),
        ],
        compiler_params=pltpu.CompilerParams(
            vmem_limit_bytes=64 * 1024 * 1024, disable_bounds_checks=True),
    )(x.reshape(B * Sq, D), k_cache.reshape(kv_shape), v_cache.reshape(kv_shape), wq, wo.T)
```

```python
import jax
import jax.numpy as jnp
from jax import lax
from jax.experimental import pallas as pl
from jax.experimental.pallas import tpu as pltpu

F32 = jnp.float32
BF16 = jnp.bfloat16
NT = (((1,), (1,)), ((), ()))

G = 2
NR = 4
RR = 512
PC = 64
NRND = RR // PC
NP = NRND * NR
NC = 8
CK = NR * RR // NC
CPH = NC // G
NS = 2 * G
NKB = 2
NVB = 4
RG = 16
OFF_HI, OFF_LO = 48, 56
WT0, WT1 = 13, 29
PLANE_ORDER = (3, 1, 2, 0)
TICKS = dict(x0=3, x1=1, x2=1, x3=1, x4=1, x5=1, x6=1, x7=1, x8=3,
             y1=2, y2=2, y3=1, y4=1, y5=1, y6=2, y7=1, y8=2, y9=2,
             c0=1, c1=1, c3=1, c5=1, c7=1)
KA = 10
VA = 10
PRO = 16
W1 = 6

KP = 0
VP = KP + NKB * NR
PP = VP + NVB * NR
NPLANES = PP + NC


def _kernel(x_hbm, k_hbm, v_hbm, wq_hbm, wot_hbm, o_hbm,
            x_buf, wq_buf, wot_buf, big, q_ref, s_ref, m_ref, l_ref, op_ref, acc_ref, o_buf,
            ksem, vsem, wsem, osem):
    B, Sq, D = o_hbm.shape
    Dh = k_hbm.shape[-1]
    H = wq_hbm.shape[1] // Dh
    N = B * H
    W = NR * RR // G
    i32 = jnp.int32
    assert sum(TICKS.values()) == NP

    def kpl(n):
        return KP + lax.rem(n, NKB) * NR

    def vpl(n):
        return VP + lax.rem(n, NVB) * NR

    def slot0(n):
        return lax.rem(lax.div(n, G) * G, NS)

    def kv_copy(src, dpl, sem, n, p0, np_, r0, cnt, c0=0, cc=None):
        srow = pl.multiple_of(lax.rem(n, G) * RR + r0, 8)
        cols = pl.ds(c0, cc or Dh)
        return pltpu.make_async_copy(
            src.at[pl.ds(lax.div(n, G) * NR + p0, np_), pl.ds(srow, cnt), cols],
            big.at[pl.ds(dpl + p0, np_), pl.ds(r0, cnt), cols], sem)

    def k_cp(n, *a):
        return kv_copy(k_hbm, kpl(n), ksem.at[lax.rem(n, NKB)], n, *a)

    def v_cp(n, *a):
        return kv_copy(v_hbm, vpl(n), vsem.at[lax.rem(n, NVB)], n, *a)

    def rows_of(r, off):
        lo = 0 if r == 0 else off + (r - 1) * PC
        hi = RR if r == NRND - 1 else off + r * PC
        return lo, hi - lo

    def piece(cp, n, t, prio):
        r, p = t // NR, PLANE_ORDER[t % NR]
        cp(n, p, 1, *rows_of(r, OFF_HI), 128, 128).start(priority=prio)
        cp(n, p, 1, *rows_of(r, OFF_LO), 0, 128).start(priority=prio)

    def wait_slot(cp, n):
        cp(n, 0, NR, 0, RR).wait()

    def o_cp(b0, cnt, s):
        return pltpu.make_async_copy(o_buf.at[pl.ds(b0, cnt)], o_hbm.at[pl.ds(b0, cnt)], osem.at[s])

    def hcol(e):
        return pl.ds(pl.multiple_of(lax.rem(e, H) * Dh, Dh), Dh)

    def chunk(pl0, j):
        return big[pl0 + j // 2, pl.ds((j % 2) * CK, CK), :]

    def qproj(e):
        x = x_buf[pl.ds(pl.multiple_of(lax.div(e, H) * Sq, 16), Sq), :]
        q = jnp.dot(x, wq_buf[:, hcol(e)], preferred_element_type=F32)
        q_ref[lax.rem(e, NS)] = (q * (Dh ** -0.5)).astype(BF16)

    def stage_x(n, tick, with_q=True):
        hs0 = slot0(n)
        q = q_ref[hs0]
        if with_q:
            qproj(n + G - 1)
        for j in range(NC):
            if j and j % CPH == 0:
                q = q_ref[hs0 + j // CPH]
            tick(f"x{j}")
            s_ref[:, pl.ds(j * CK, CK)] = lax.dot_general(
                q, chunk(kpl(n), j), NT, preferred_element_type=F32)
        tick("x8")

    def c_group(n, g, pp, heads=range(G)):
        hs0 = slot0(n)
        u = lax.rem(n, G)
        rows = pl.ds(g * RG, RG)
        for a in heads:
            s = s_ref[rows, pl.ds(a * W, W)]
            m = jnp.max(s, axis=-1, keepdims=True)
            p = jnp.exp(s - m)
            lp = p[:, :128]
            for c in range(1, W // 128):
                lp = lp + p[:, c * 128:(c + 1) * 128]
            m_ref[hs0 + a, u, rows, :] = jnp.broadcast_to(m, (RG, 128))
            l_ref[hs0 + a, u, rows, :] = lp
            pb = p.astype(BF16)
            for jj in range(CPH):
                big[pp + a * CPH + jj, rows, :] = pb[:, jj * CK:(jj + 1) * CK]

    def stage_c(n, tick):
        for g in range(Sq // RG):
            c_group(n, g, PP)
            tick(f"c{g}")

    def merge(e):
        hs = lax.rem(e + NS, NS)
        m0, m1 = m_ref[hs, 0], m_ref[hs, 1]
        mx = jnp.maximum(m0, m1)
        a0, a1 = jnp.exp(m0 - mx), jnp.exp(m1 - mx)
        r = 1.0 / jnp.sum(a0 * l_ref[hs, 0] + a1 * l_ref[hs, 1], axis=-1, keepdims=True)
        w0, w1 = a0 * r, a1 * r
        o = (op_ref[hs, 0] * jnp.concatenate([w0, w0], axis=1)
             + op_ref[hs, 1] * jnp.concatenate([w1, w1], axis=1))
        return o.astype(BF16)

    def outproj(e, o):
        acc_ref[...] += lax.dot_general(
            o, wot_buf[:, hcol(jnp.maximum(e, 0))], NT, preferred_element_type=F32)

    def stage_y(n, tick, pp=PP):
        hs0 = slot0(n)
        u = lax.rem(n, G)
        v_next = chunk(vpl(n), 0)
        for j in range(NC):
            tick(f"y{j + 1}")
            vj = v_next
            if j + 1 < NC:
                v_next = chunk(vpl(n), j + 1)
            oj = jnp.dot(big[pp + j, pl.ds(0, Sq), :], vj, preferred_element_type=F32)
            o = oj if j % CPH == 0 else o + oj
            if j % CPH == CPH - 1:
                op_ref[hs0 + j // CPH, u] = o
            if j == CPH - 1:
                merged = merge(n - 1)
        tick("y9")
        outproj(n - 1, merged)

    XR = 32
    NX = (B * Sq) // XR
    NWG = D // 8

    def x_piece(t):
        t = lax.rem(t, 2) * (NX // 2) + lax.div(t, 2)
        r = pl.ds(pl.multiple_of(t * XR, XR), XR)
        return pltpu.make_async_copy(x_hbm.at[r], x_buf.at[r], wsem.at[2])

    def plain_piece(cp, n, t):
        return cp(n, lax.rem(t, NR), 1, pl.multiple_of(lax.div(t, NR) * PC, 8), PC)

    def load_k0_x(t, c):
        plain_piece(k_cp, i32(0), t).start(priority=0)
        x_piece(t).start(priority=1)
        return c

    def load_x(t, c):
        x_piece(t).start(priority=1)
        return c

    def load_w(t, c):
        def w_cp(src, dst, sem, group, t0, t1):
            r = pl.ds(pl.multiple_of(group * 8, 8), 8)
            cols = pl.ds(t0 * 128, (t1 - t0) * 128)
            return pltpu.make_async_copy(src.at[r, cols], dst.at[r, cols], sem)

        both = ((wq_hbm, wq_buf, wsem.at[0], 0), (wot_hbm, wot_buf, wsem.at[1], 1))
        for p in range(NR):
            for src, dst, sem, prio in both:
                w_cp(src, dst, sem, p * (NWG // NR) + t, WT0, WT1).start(priority=prio)
        for p in range(NR):
            group = p * (NWG // NR) + t
            nxt = jnp.where(group + 1 == NWG, 0, group + 1)
            for src, dst, sem, prio in both:
                w_cp(src, dst, sem, group, WT1, H * Dh // 128).start(priority=prio)
                w_cp(src, dst, sem, nxt, 0, WT0).start(priority=prio)
        return c

    def load_k1_v0(t, c):
        plain_piece(k_cp, i32(1), t).start(priority=0)
        plain_piece(v_cp, i32(0), t).start(priority=1)
        return c

    lax.fori_loop(0, 24, load_k0_x, 0)
    acc_ref[...] = jnp.zeros_like(acc_ref)
    op_ref[NS - 1] = jnp.zeros(op_ref.shape[1:], F32)
    m_ref[NS - 1] = jnp.zeros(m_ref.shape[1:], F32)
    l_ref[NS - 1] = jnp.ones(l_ref.shape[1:], F32)
    lax.fori_loop(24, NP, load_k0_x, 0)
    lax.fori_loop(NP, NX, load_x, 0)
    lax.fori_loop(0, NWG // NR, load_w, 0)
    lax.fori_loop(0, NP - PRO, load_k1_v0, 0)
    pltpu.make_async_copy(wq_hbm, wq_buf, wsem.at[0]).wait()
    pltpu.make_async_copy(x_hbm, x_buf, wsem.at[2]).wait()
    wait_slot(k_cp, i32(0))

    todo = list(range(NP - PRO, NP))

    def pro_tick_x(name):
        for _ in range(2):
            if todo:
                load_k1_v0(i32(todo.pop(0)), 0)

    qproj(i32(0))
    stage_x(i32(0), pro_tick_x)
    assert not todo
    todo = list(range(max(KA, VA)))

    def pro_tick_c(name):
        for _ in range(2):
            if todo:
                t = todo.pop(0)
                if t < KA:
                    piece(k_cp, i32(2), t, 0)
                if t < VA:
                    piece(v_cp, i32(1), t, 1)

    pro_tick_c("pre")
    stage_c(i32(0), pro_tick_c)
    assert not todo
    pltpu.make_async_copy(wot_hbm, wot_buf, wsem.at[1]).wait()

    def iteration(i, carry):
        started = [0]

        def tick(name):
            for _ in range(TICKS.get(name, 0)):
                t = started[0]
                started[0] += 1
                dk, tk = divmod(t + KA, NP)
                if dk == 0:
                    piece(k_cp, i + 2, tk, 0)
                else:
                    @pl.when(i + 3 < N)
                    def _():
                        piece(k_cp, i + 3, tk, 0)
                dv, tv = divmod(t + VA, NP)
                piece(v_cp, i + 1 + dv, tv, 1)

        wait_slot(k_cp, i + 1)
        stage_x(i + 1, tick)
        wait_slot(v_cp, i)
        stage_y(i, tick)
        stage_c(i + 1, tick)
        assert started[0] == NP

        @pl.when(jnp.logical_and(i > 0, lax.rem(i, H) == 0))
        def _():
            o_buf[lax.div(i, H) - 1] = acc_ref[...].astype(o_buf.dtype)
            acc_ref[...] = jnp.zeros_like(acc_ref)

        return carry

    lax.fori_loop(0, N - 2, iteration, 0)

    todo = list(range(VA, NP))

    def tail_tick_x(name):
        for prio in (0, 1, 0, 1):
            if todo:
                piece(v_cp, i32(N - 1), todo.pop(0), prio)

    def tail_tick_y(name):
        if name == "y9":
            o_buf[B - 1, pl.ds(0, RG), pl.ds(0, Dh)] = (
                op_ref[(N - 1) % NS, 0, pl.ds(0, RG), :].astype(o_buf.dtype))
            o_cp(0, W1, 0).start(priority=1)

    def no_tick(name):
        pass

    wait_slot(k_cp, i32(N - 1))
    stage_x(i32(N - 1), tail_tick_x, with_q=False)
    assert not todo
    for g in range(Sq // RG):
        c_group(i32(N - 1), g, KP, [0])
    wait_slot(v_cp, i32(N - 2))
    stage_y(i32(N - 2), tail_tick_y)
    for g in range(Sq // RG):
        c_group(i32(N - 1), g, KP, [1])
    wait_slot(v_cp, i32(N - 1))
    o_cp(W1, B - 1 - W1, 1).start(priority=1)
    stage_y(i32(N - 1), no_tick, KP)
    o = merge(i32(N - 1))
    last = []
    for k, (c0, cc) in enumerate(((0, 256), (256, D - 256))):
        cols = pl.ds(c0, cc)
        y = lax.dot_general(o, wot_buf[cols, hcol(i32(N - 1))], NT, preferred_element_type=F32)
        o_buf[B - 1, :, cols] = (acc_ref[:, cols] + y).astype(o_buf.dtype)
        last.append(pltpu.make_async_copy(
            o_buf.at[B - 1, :, cols], o_hbm.at[B - 1, :, cols], osem.at[2 + k]))
        last[-1].start(priority=0)
    o_cp(0, W1, 0).wait()
    o_cp(W1, B - 1 - W1, 1).wait()
    for c in last:
        c.wait()


@jax.jit
def pallas_standalone__mha_block_cached__near_ridge_kernel(
    x: jax.Array,
    k_cache: jax.Array,
    v_cache: jax.Array,
    wq: jax.Array,
    wo: jax.Array,
):
    B, Sq, D = x.shape
    _, H, Sk, Dh = k_cache.shape
    assert Sk == NR * RR and Dh == 256 and H % G == 0 and Sq % RG == 0
    assert H * Dh > WT1 * 128 and D % (8 * NR) == 0 and D > 256 and B > W1 + 1
    assert (B * Sq) % 64 == 0 and (B * Sq) // 32 >= NP
    in_hbm = pl.BlockSpec(memory_space=pl.ANY)
    kv_shape = (B * H * NR // G, RR * G, Dh)
    return pl.pallas_call(
        _kernel,
        in_specs=[in_hbm] * 5,
        out_specs=in_hbm,
        out_shape=jax.ShapeDtypeStruct((B, Sq, D), x.dtype),
        scratch_shapes=[
            pltpu.VMEM((B * Sq, D), BF16),
            pltpu.VMEM((D, H * Dh), BF16),
            pltpu.VMEM((D, H * Dh), BF16),
            pltpu.VMEM((NPLANES, RR, Dh), BF16),
            pltpu.VMEM((NS, Sq, Dh), BF16),
            pltpu.VMEM((Sq, Sk), F32),
            pltpu.VMEM((NS, G, Sq, 128), F32),
            pltpu.VMEM((NS, G, Sq, 128), F32),
            pltpu.VMEM((NS, G, Sq, Dh), F32),
            pltpu.VMEM((Sq, D), F32),
            pltpu.VMEM((B, Sq, D), BF16),
            pltpu.SemaphoreType.DMA((NKB,)),
            pltpu.SemaphoreType.DMA((NVB,)),
            pltpu.SemaphoreType.DMA((3,)),
            pltpu.SemaphoreType.DMA((4,)),
        ],
        compiler_params=pltpu.CompilerParams(
            vmem_limit_bytes=64 * 1024 * 1024, disable_bounds_checks=True),
    )(x.reshape(B * Sq, D), k_cache.reshape(kv_shape), v_cache.reshape(kv_shape), wq, wo.T)
```

```python
import jax
import jax.numpy as jnp
from jax import lax
from jax.experimental import pallas as pl
from jax.experimental.pallas import tpu as pltpu

F32 = jnp.float32
BF16 = jnp.bfloat16
NT = (((1,), (1,)), ((), ()))

G = 2
NR = 4
RR = 512
PC = 64
NRND = RR // PC
NP = NRND * NR
NC = 8
CK = NR * RR // NC
CPH = NC // G
NS = 2 * G
NKB = 2
NVB = 4
RG = 16
OFF_HI, OFF_LO = 48, 56
WT0, WT1 = 13, 29
PLANE_ORDER = (3, 1, 2, 0)
TICKS = dict(x0=3, x1=1, x2=1, x3=1, x4=1, x5=1, x6=1, x7=1, x8=3,
             y1=2, y2=2, y3=1, y4=1, y5=1, y6=2, y7=1, y8=2, y9=2,
             c0=1, c1=1, c3=1, c5=1, c7=1)
KA = 11
VA = 9
PRO = 16

KP = 0
VP = KP + NKB * NR
PP = VP + NVB * NR
NPLANES = PP + NC


def _kernel(x_hbm, k_hbm, v_hbm, wq_hbm, wot_hbm, o_hbm,
            x_buf, wq_buf, wot_buf, big, q_ref, s_ref, m_ref, l_ref, op_ref, acc_ref, o_buf,
            ksem, vsem, wsem, osem):
    B, Sq, D = o_hbm.shape
    Dh = k_hbm.shape[-1]
    H = wq_hbm.shape[1] // Dh
    N = B * H
    W = NR * RR // G
    i32 = jnp.int32
    assert sum(TICKS.values()) == NP

    def kpl(n):
        return KP + lax.rem(n, NKB) * NR

    def vpl(n):
        return VP + lax.rem(n, NVB) * NR

    def slot0(n):
        return lax.rem(lax.div(n, G) * G, NS)

    def head_of(e):
        return lax.rem(lax.div(e, G), H)

    def batch_of(e):
        return lax.div(e, G * H) * G + lax.rem(e, G)

    def kv_copy(src, dpl, sem, n, p, r0, cnt, c0=0, cc=None):
        spl = ((lax.div(n, G * H) * G + p // 2) * H + head_of(n)) * 2 + p % 2
        srow = pl.multiple_of(lax.rem(n, G) * RR + r0, 8)
        cols = pl.ds(c0, cc or Dh)
        return pltpu.make_async_copy(
            src.at[spl, pl.ds(srow, cnt), cols], big.at[dpl + p, pl.ds(r0, cnt), cols], sem)

    def k_cp(n, *a):
        return kv_copy(k_hbm, kpl(n), ksem.at[lax.rem(n, NKB)], n, *a)

    def v_cp(n, *a):
        return kv_copy(v_hbm, vpl(n), vsem.at[lax.rem(n, NVB)], n, *a)

    def rows_of(r, off):
        lo = 0 if r == 0 else off + (r - 1) * PC
        hi = RR if r == NRND - 1 else off + r * PC
        return lo, hi - lo

    def piece(cp, n, t, prio):
        r, p = t // NR, PLANE_ORDER[t % NR]
        cp(n, p, *rows_of(r, OFF_HI), 128, 128).start(priority=prio)
        cp(n, p, *rows_of(r, OFF_LO), 0, 128).start(priority=prio)

    def wait_slot(pl0, sem):
        slot = big.at[pl.ds(pl0, NR)]
        pltpu.make_async_copy(slot, slot, sem).wait()

    def wait_k(n):
        wait_slot(kpl(n), ksem.at[lax.rem(n, NKB)])

    def wait_v(n):
        wait_slot(vpl(n), vsem.at[lax.rem(n, NVB)])

    def o_cp(b0, cnt, s):
        return pltpu.make_async_copy(o_buf.at[pl.ds(b0, cnt)], o_hbm.at[pl.ds(b0, cnt)], osem.at[s])

    def hcol(e):
        return pl.ds(pl.multiple_of(head_of(e) * Dh, Dh), Dh)

    def chunk(pl0, j):
        return big[pl0 + j // 2, pl.ds((j % 2) * CK, CK), :]

    def qproj(e):
        x = x_buf[pl.ds(pl.multiple_of(batch_of(e) * Sq, 16), Sq), :]
        q = jnp.dot(x, wq_buf[:, hcol(e)], preferred_element_type=F32)
        q_ref[lax.rem(e, NS)] = (q * (Dh ** -0.5)).astype(BF16)

    def stage_x(n, tick, with_q=True):
        hs0 = slot0(n)
        q = q_ref[hs0]
        if with_q:
            qproj(n + G - 1)
        for j in range(NC):
            if j and j % CPH == 0:
                q = q_ref[hs0 + j // CPH]
            tick(f"x{j}")
            s_ref[:, pl.ds(j * CK, CK)] = lax.dot_general(
                q, chunk(kpl(n), j), NT, preferred_element_type=F32)
        tick("x8")

    def c_group(n, g, pp, items=range(G)):
        hs0 = slot0(n)
        u = lax.rem(n, G)
        rows = pl.ds(g * RG, RG)
        for a in items:
            s = s_ref[rows, pl.ds(a * W, W)]
            m = jnp.max(s, axis=-1, keepdims=True)
            p = jnp.exp(s - m)
            lp = p[:, :128]
            for c in range(1, W // 128):
                lp = lp + p[:, c * 128:(c + 1) * 128]
            m_ref[hs0 + a, u, rows, :] = jnp.broadcast_to(m, (RG, 128))
            l_ref[hs0 + a, u, rows, :] = lp
            pb = p.astype(BF16)
            for jj in range(CPH):
                big[pp + a * CPH + jj, rows, :] = pb[:, jj * CK:(jj + 1) * CK]

    def stage_c(n, tick):
        for g in range(Sq // RG):
            c_group(n, g, PP)
            tick(f"c{g}")

    def merge(e):
        hs = lax.rem(e + NS, NS)
        m0, m1 = m_ref[hs, 0], m_ref[hs, 1]
        mx = jnp.maximum(m0, m1)
        a0, a1 = jnp.exp(m0 - mx), jnp.exp(m1 - mx)
        r = 1.0 / jnp.sum(a0 * l_ref[hs, 0] + a1 * l_ref[hs, 1], axis=-1, keepdims=True)
        w0, w1 = a0 * r, a1 * r
        o = (op_ref[hs, 0] * jnp.concatenate([w0, w0], axis=1)
             + op_ref[hs, 1] * jnp.concatenate([w1, w1], axis=1))
        return o.astype(BF16)

    def outproj(e, o):
        e = jnp.maximum(e, 0)
        acc_ref[lax.rem(e, G)] += lax.dot_general(
            o, wot_buf[:, hcol(e)], NT, preferred_element_type=F32)

    def stage_y(n, tick, pp=PP, finish=outproj):
        hs0 = slot0(n)
        u = lax.rem(n, G)
        v_next = chunk(vpl(n), 0)
        for j in range(NC):
            tick(f"y{j + 1}")
            vj = v_next
            if j + 1 < NC:
                v_next = chunk(vpl(n), j + 1)
            oj = jnp.dot(big[pp + j, pl.ds(0, Sq), :], vj, preferred_element_type=F32)
            o = oj if j % CPH == 0 else o + oj
            if j % CPH == CPH - 1:
                op_ref[hs0 + j // CPH, u] = o
            if j == CPH - 1:
                merged = merge(n - 1)
        tick("y9")
        finish(n - 1, merged)

    XR = 32
    NX = (B * Sq) // XR
    NWG = D // 8

    def x_piece(t):
        t = lax.rem(t, 2) * (NX // 2) + lax.div(t, 2)
        r = pl.ds(pl.multiple_of(t * XR, XR), XR)
        return pltpu.make_async_copy(x_hbm.at[r], x_buf.at[r], wsem.at[2])

    def plain_piece(cp, n, t):
        return cp(n, NR - 1 - lax.rem(t, NR), pl.multiple_of(lax.div(t, NR) * PC, 8), PC)

    def load_k0_x(t, c):
        plain_piece(k_cp, i32(0), t).start(priority=0)
        x_piece(t).start(priority=1)
        return c

    def load_x(t, c):
        x_piece(t).start(priority=1)
        return c

    def load_w(t, c):
        def w_cp(src, dst, sem, group, t0, t1):
            r = pl.ds(pl.multiple_of(group * 8, 8), 8)
            cols = pl.ds(t0 * 128, (t1 - t0) * 128)
            return pltpu.make_async_copy(src.at[r, cols], dst.at[r, cols], sem)

        both = ((wq_hbm, wq_buf, wsem.at[0], 0), (wot_hbm, wot_buf, wsem.at[1], 1))
        for p in range(NR):
            for src, dst, sem, prio in both:
                w_cp(src, dst, sem, p * (NWG // NR) + t, WT0, WT1).start(priority=prio)
        for p in range(NR):
            group = p * (NWG // NR) + t
            nxt = jnp.where(group + 1 == NWG, 0, group + 1)
            for src, dst, sem, prio in both:
                w_cp(src, dst, sem, group, WT1, H * Dh // 128).start(priority=prio)
                w_cp(src, dst, sem, nxt, 0, WT0).start(priority=prio)
        return c

    def load_k1_v0(t, c):
        plain_piece(k_cp, i32(1), t).start(priority=0)
        plain_piece(v_cp, i32(0), t).start(priority=1)
        return c

    lax.fori_loop(0, 24, load_k0_x, 0)
    acc_ref[...] = jnp.zeros_like(acc_ref)
    op_ref[NS - 1] = jnp.zeros(op_ref.shape[1:], F32)
    m_ref[NS - 1] = jnp.zeros(m_ref.shape[1:], F32)
    l_ref[NS - 1] = jnp.ones(l_ref.shape[1:], F32)
    lax.fori_loop(24, NP, load_k0_x, 0)
    lax.fori_loop(NP, NX, load_x, 0)
    lax.fori_loop(0, NWG // NR, load_w, 0)
    lax.fori_loop(0, NP - PRO, load_k1_v0, 0)
    pltpu.make_async_copy(wq_hbm, wq_buf, wsem.at[0]).wait()
    pltpu.make_async_copy(x_hbm, x_buf, wsem.at[2]).wait()
    wait_k(i32(0))

    todo = list(range(NP - PRO, NP))

    def pro_tick_x(name):
        for _ in range(2):
            if todo:
                load_k1_v0(i32(todo.pop(0)), 0)

    qproj(i32(0))
    stage_x(i32(0), pro_tick_x)
    assert not todo
    todo = list(range(max(KA, VA)))

    def pro_tick_c(name):
        for _ in range(2):
            if todo:
                t = todo.pop(0)
                if t < KA:
                    piece(k_cp, i32(2), t, 0)
                if t < VA:
                    piece(v_cp, i32(1), t, 1)

    pro_tick_c("pre")
    stage_c(i32(0), pro_tick_c)
    assert not todo
    pltpu.make_async_copy(wot_hbm, wot_buf, wsem.at[1]).wait()

    def iteration(i, carry):
        started = [0]

        def tick(name):
            for _ in range(TICKS.get(name, 0)):
                t = started[0]
                started[0] += 1
                dk, tk = divmod(t + KA, NP)
                if dk == 0:
                    piece(k_cp, i + 2, tk, 0)
                else:
                    @pl.when(i + 3 < N)
                    def _():
                        piece(k_cp, i + 3, tk, 0)
                dv, tv = divmod(t + VA, NP)
                piece(v_cp, i + 1 + dv, tv, 1)

        wait_k(i + 1)
        stage_x(i + 1, tick)
        wait_v(i)
        stage_y(i, tick)
        stage_c(i + 1, tick)
        assert started[0] == NP

        e = jnp.maximum(i - 1, 0)

        @pl.when(head_of(e) == H - 1)
        def _():
            o_buf[batch_of(e)] = acc_ref[lax.rem(e, G)].astype(o_buf.dtype)
            acc_ref[lax.rem(e, G)] = jnp.zeros(acc_ref.shape[1:], F32)

        return carry

    lax.fori_loop(0, N - 2, iteration, 0)

    todo = list(range(VA, NP))

    def tail_tick_x(name):
        for prio in (0, 1, 0, 1):
            if todo:
                piece(v_cp, i32(N - 1), todo.pop(0), prio)

    def tail_tick_y(name):
        if name == "y9":
            o_buf[B - 1, pl.ds(0, RG), pl.ds(0, Dh)] = (
                op_ref[(N - 1) % NS, 0, pl.ds(0, RG), :].astype(o_buf.dtype))
            o_cp(0, B - G, 0).start(priority=1)

    def no_tick(name):
        pass

    wait_k(i32(N - 1))
    stage_x(i32(N - 1), tail_tick_x, with_q=False)
    assert not todo
    for g in range(Sq // RG):
        c_group(i32(N - 1), g, KP, [0])
    wait_v(i32(N - 2))
    stage_y(i32(N - 2), tail_tick_y)
    for g in range(Sq // RG):
        c_group(i32(N - 1), g, KP, [1])
    wait_v(i32(N - 1))
    last = []

    def finish_batch(e, o):
        a = len(last) // 2
        for c0, cc in ((0, 256), (256, D - 256)):
            cols = pl.ds(c0, cc)
            y = lax.dot_general(o, wot_buf[cols, hcol(e)], NT, preferred_element_type=F32)
            o_buf[B - G + a, :, cols] = (acc_ref[a, :, cols] + y).astype(o_buf.dtype)
            last.append(pltpu.make_async_copy(
                o_buf.at[B - G + a, :, cols], o_hbm.at[B - G + a, :, cols], osem.at[1 + len(last)]))
            last[-1].start(priority=0)

    stage_y(i32(N - 1), no_tick, KP, finish_batch)
    finish_batch(i32(N - 1), merge(i32(N - 1)))
    o_cp(0, B - G, 0).wait()
    for c in last:
        c.wait()


@jax.jit
def pallas_standalone__mha_block_cached__near_ridge_kernel(
    x: jax.Array,
    k_cache: jax.Array,
    v_cache: jax.Array,
    wq: jax.Array,
    wo: jax.Array,
):
    B, Sq, D = x.shape
    _, H, Sk, Dh = k_cache.shape
    assert Sk == NR * RR and Dh == 256 and B % G == 0 and Sq % RG == 0
    assert H * Dh > WT1 * 128 and D % (8 * NR) == 0 and D > 256 and B > G
    assert (B * Sq) % 64 == 0 and (B * Sq) // 32 >= NP
    in_hbm = pl.BlockSpec(memory_space=pl.ANY)
    kv_shape = (B * H * NR // G, RR * G, Dh)
    return pl.pallas_call(
        _kernel,
        in_specs=[in_hbm] * 5,
        out_specs=in_hbm,
        out_shape=jax.ShapeDtypeStruct((B, Sq, D), x.dtype),
        scratch_shapes=[
            pltpu.VMEM((B * Sq, D), BF16),
            pltpu.VMEM((D, H * Dh), BF16),
            pltpu.VMEM((D, H * Dh), BF16),
            pltpu.VMEM((NPLANES, RR, Dh), BF16),
            pltpu.VMEM((NS, Sq, Dh), BF16),
            pltpu.VMEM((Sq, Sk), F32),
            pltpu.VMEM((NS, G, Sq, 128), F32),
            pltpu.VMEM((NS, G, Sq, 128), F32),
            pltpu.VMEM((NS, G, Sq, Dh), F32),
            pltpu.VMEM((G, Sq, D), F32),
            pltpu.VMEM((B, Sq, D), BF16),
            pltpu.SemaphoreType.DMA((NKB,)),
            pltpu.SemaphoreType.DMA((NVB,)),
            pltpu.SemaphoreType.DMA((3,)),
            pltpu.SemaphoreType.DMA((5,)),
        ],
        compiler_params=pltpu.CompilerParams(
            vmem_limit_bytes=64 * 1024 * 1024, disable_bounds_checks=True),
    )(x.reshape(B * Sq, D), k_cache.reshape(kv_shape), v_cache.reshape(kv_shape), wq, wo.T)
```

```python
import jax
import jax.numpy as jnp
from jax import lax
from jax.experimental import pallas as pl
from jax.experimental.pallas import tpu as pltpu

F32 = jnp.float32
BF16 = jnp.bfloat16
NT = (((1,), (1,)), ((), ()))

G = 2
NR = 4
RR = 512
PC = 64
NRND = RR // PC
NP = NRND * NR
NC = 8
CK = NR * RR // NC
CPH = NC // G
NS = 2 * G
NKB = 2
NVB = 4
RG = 16
OFF_HI, OFF_LO = 48, 56
WT0, WT1 = 13, 29
PLANE_ORDER = (3, 1, 2, 0)
TICKS = dict(x0=3, x1=1, x2=1, x3=1, x4=1, x5=1, x6=1, x7=1, x8=3,
             y1=2, y2=2, y3=1, y4=1, y5=1, y6=2, y7=1, y8=2, y9=2,
             c0=1, c1=1, c3=1, c5=1, c7=1)
KA = 11
VA = 9
PRO = 16

KP = 0
VP = KP + NKB * NR
PP = VP + NVB * NR
NPLANES = PP + NC


def _kernel(x_hbm, k_hbm, v_hbm, wq_hbm, wot_hbm, o_hbm,
            x_buf, wq_buf, wot_buf, big, q_ref, s_ref, m_ref, l_ref, op_ref, acc_ref, o_buf,
            ksem, vsem, wsem, osem):
    B, Sq, D = o_hbm.shape
    Dh = k_hbm.shape[-1]
    H = wq_hbm.shape[1] // Dh
    N = B * H
    W = NR * RR // G
    i32 = jnp.int32
    assert sum(TICKS.values()) == NP

    def kpl(n):
        return KP + lax.rem(n, NKB) * NR

    def vpl(n):
        return VP + lax.rem(n, NVB) * NR

    def slot0(n):
        return lax.rem(lax.div(n, G) * G, NS)

    def head_of(e):
        return lax.rem(lax.div(e, G), H)

    def batch_of(e):
        return lax.div(e, G * H) * G + lax.rem(e, G)

    def kv_copier(src, dpl, sem, n):
        spl = (lax.div(n, G * H) * (G * H) + head_of(n)) * 2
        srow = lax.rem(n, G) * RR

        def copy(p, r0, cnt, c0=0, cc=Dh):
            cols = pl.ds(c0, cc)
            return pltpu.make_async_copy(
                src.at[spl + (p // 2 * (2 * H) + p % 2), pl.ds(pl.multiple_of(srow + r0, 8), cnt), cols],
                big.at[dpl + p, pl.ds(r0, cnt), cols], sem)

        return copy

    def k_cp(n):
        return kv_copier(k_hbm, kpl(n), ksem.at[lax.rem(n, NKB)], n)

    def v_cp(n):
        return kv_copier(v_hbm, vpl(n), vsem.at[lax.rem(n, NVB)], n)

    def rows_of(r, off):
        lo = 0 if r == 0 else off + (r - 1) * PC
        hi = RR if r == NRND - 1 else off + r * PC
        return lo, hi - lo

    def piece(cp, t, prio):
        r, p = t // NR, PLANE_ORDER[t % NR]
        cp(p, *rows_of(r, OFF_HI), 128, 128).start(priority=prio)
        cp(p, *rows_of(r, OFF_LO), 0, 128).start(priority=prio)

    def wait_slot(pl0, sem):
        slot = big.at[pl.ds(pl0, NR)]
        pltpu.make_async_copy(slot, slot, sem).wait()

    def wait_k(n):
        wait_slot(kpl(n), ksem.at[lax.rem(n, NKB)])

    def wait_v(n):
        wait_slot(vpl(n), vsem.at[lax.rem(n, NVB)])

    def o_cp(b0, cnt, s):
        return pltpu.make_async_copy(o_buf.at[pl.ds(b0, cnt)], o_hbm.at[pl.ds(b0, cnt)], osem.at[s])

    def hcol(e):
        return pl.ds(pl.multiple_of(head_of(e) * Dh, Dh), Dh)

    def chunk(pl0, j):
        return big[pl0 + j // 2, pl.ds((j % 2) * CK, CK), :]

    def qproj(e):
        x = x_buf[pl.ds(pl.multiple_of(batch_of(e) * Sq, 16), Sq), :]
        q = jnp.dot(x, wq_buf[:, hcol(e)], preferred_element_type=F32)
        q_ref[lax.rem(e, NS)] = (q * (Dh ** -0.5)).astype(BF16)

    def stage_x(n, tick, with_q=True):
        hs0 = slot0(n)
        kp = kpl(n)
        q = q_ref[hs0]
        if with_q:
            qproj(n + G - 1)
        for j in range(NC):
            if j and j % CPH == 0:
                q = q_ref[hs0 + j // CPH]
            tick(f"x{j}")
            s_ref[:, pl.ds(j * CK, CK)] = lax.dot_general(
                q, chunk(kp, j), NT, preferred_element_type=F32)
        tick("x8")

    def c_group(n, g, pp, items=range(G)):
        hs0 = slot0(n)
        u = lax.rem(n, G)
        rows = pl.ds(g * RG, RG)
        for a in items:
            s = s_ref[rows, pl.ds(a * W, W)]
            m = jnp.max(s, axis=-1, keepdims=True)
            p = jnp.exp(s - m)
            lp = p[:, :128]
            for c in range(1, W // 128):
                lp = lp + p[:, c * 128:(c + 1) * 128]
            m_ref[hs0 + a, u, rows, :] = jnp.broadcast_to(m, (RG, 128))
            l_ref[hs0 + a, u, rows, :] = lp
            pb = p.astype(BF16)
            for jj in range(CPH):
                big[pp + a * CPH + jj, rows, :] = pb[:, jj * CK:(jj + 1) * CK]

    def stage_c(n, tick):
        for g in range(Sq // RG):
            c_group(n, g, PP)
            tick(f"c{g}")

    def merge(e):
        hs = lax.rem(e + NS, NS)
        m0, m1 = m_ref[hs, 0], m_ref[hs, 1]
        mx = jnp.maximum(m0, m1)
        a0, a1 = jnp.exp(m0 - mx), jnp.exp(m1 - mx)
        r = 1.0 / jnp.sum(a0 * l_ref[hs, 0] + a1 * l_ref[hs, 1], axis=-1, keepdims=True)
        w0, w1 = a0 * r, a1 * r
        o = (op_ref[hs, 0] * jnp.concatenate([w0, w0], axis=1)
             + op_ref[hs, 1] * jnp.concatenate([w1, w1], axis=1))
        return o.astype(BF16)

    def outproj(e, o):
        e = jnp.maximum(e, 0)
        acc_ref[lax.rem(e, G)] += lax.dot_general(
            o, wot_buf[:, hcol(e)], NT, preferred_element_type=F32)

    def stage_y(n, tick, pp=PP, finish=outproj):
        hs0 = slot0(n)
        u = lax.rem(n, G)
        vp = vpl(n)
        v_next = chunk(vp, 0)
        for j in range(NC):
            tick(f"y{j + 1}")
            vj = v_next
            if j + 1 < NC:
                v_next = chunk(vp, j + 1)
            oj = jnp.dot(big[pp + j, pl.ds(0, Sq), :], vj, preferred_element_type=F32)
            o = oj if j % CPH == 0 else o + oj
            if j % CPH == CPH - 1:
                op_ref[hs0 + j // CPH, u] = o
            if j == CPH - 1:
                merged = merge(n - 1)
        tick("y9")
        finish(n - 1, merged)

    XR = 32
    NX = (B * Sq) // XR
    NWG = D // 8

    def x_piece(t):
        t = lax.rem(t, 2) * (NX // 2) + lax.div(t, 2)
        r = pl.ds(pl.multiple_of(t * XR, XR), XR)
        return pltpu.make_async_copy(x_hbm.at[r], x_buf.at[r], wsem.at[2])

    def plain_piece(cp, t):
        return cp(NR - 1 - lax.rem(t, NR), pl.multiple_of(lax.div(t, NR) * PC, 8), PC)

    k0, k1, k2, v0, v1 = k_cp(i32(0)), k_cp(i32(1)), k_cp(i32(2)), v_cp(i32(0)), v_cp(i32(1))

    def load_k0_x(t, c):
        plain_piece(k0, t).start(priority=0)
        x_piece(t).start(priority=1)
        return c

    def load_x(t, c):
        x_piece(t).start(priority=1)
        return c

    def load_w(t, c):
        def w_cp(src, dst, sem, group, t0, t1):
            r = pl.ds(pl.multiple_of(group * 8, 8), 8)
            cols = pl.ds(t0 * 128, (t1 - t0) * 128)
            return pltpu.make_async_copy(src.at[r, cols], dst.at[r, cols], sem)

        both = ((wq_hbm, wq_buf, wsem.at[0], 0), (wot_hbm, wot_buf, wsem.at[1], 1))
        for p in range(NR):
            for src, dst, sem, prio in both:
                w_cp(src, dst, sem, p * (NWG // NR) + t, WT0, WT1).start(priority=prio)
        for p in range(NR):
            group = p * (NWG // NR) + t
            nxt = jnp.where(group + 1 == NWG, 0, group + 1)
            for src, dst, sem, prio in both:
                w_cp(src, dst, sem, group, WT1, H * Dh // 128).start(priority=prio)
                w_cp(src, dst, sem, nxt, 0, WT0).start(priority=prio)
        return c

    def load_k1_v0(t, c):
        plain_piece(k1, t).start(priority=0)
        plain_piece(v0, t).start(priority=1)
        return c

    lax.fori_loop(0, 24, load_k0_x, 0)
    acc_ref[...] = jnp.zeros_like(acc_ref)
    op_ref[NS - 1] = jnp.zeros(op_ref.shape[1:], F32)
    m_ref[NS - 1] = jnp.zeros(m_ref.shape[1:], F32)
    l_ref[NS - 1] = jnp.ones(l_ref.shape[1:], F32)
    lax.fori_loop(24, NP, load_k0_x, 0)
    lax.fori_loop(NP, NX, load_x, 0)
    lax.fori_loop(0, NWG // NR, load_w, 0)
    lax.fori_loop(0, NP - PRO, load_k1_v0, 0)
    pltpu.make_async_copy(wq_hbm, wq_buf, wsem.at[0]).wait()
    pltpu.make_async_copy(x_hbm, x_buf, wsem.at[2]).wait()
    wait_k(i32(0))

    todo = list(range(NP - PRO, NP))

    def pro_tick_x(name):
        for _ in range(2):
            if todo:
                load_k1_v0(i32(todo.pop(0)), 0)

    qproj(i32(0))
    stage_x(i32(0), pro_tick_x)
    assert not todo
    todo = list(range(max(KA, VA)))

    def pro_tick_c(name):
        for _ in range(2):
            if todo:
                t = todo.pop(0)
                if t < KA:
                    piece(k2, t, 0)
                if t < VA:
                    piece(v1, t, 1)

    pro_tick_c("pre")
    stage_c(i32(0), pro_tick_c)
    assert not todo
    pltpu.make_async_copy(wot_hbm, wot_buf, wsem.at[1]).wait()

    def iteration(i, carry):
        started = [0]

        def tick(name):
            for _ in range(TICKS.get(name, 0)):
                t = started[0]
                started[0] += 1
                dk, tk = divmod(t + KA, NP)
                if dk == 0:
                    piece(k_now, tk, 0)
                else:
                    assert name[0] != "x"

                    @pl.when(has_next)
                    def _():
                        piece(k_next, tk, 0)
                dv, tv = divmod(t + VA, NP)
                piece(v_next if dv else v_now, tv, 1)

        wait_k(i + 1)
        k_now, v_now = k_cp(i + 2), v_cp(i + 1)
        stage_x(i + 1, tick)
        wait_v(i)
        k_next, v_next, has_next = k_cp(i + 3), v_cp(i + 2), i + 3 < N
        stage_y(i, tick)
        stage_c(i + 1, tick)
        assert started[0] == NP

        e = jnp.maximum(i - 1, 0)

        @pl.when(head_of(e) == H - 1)
        def _():
            o_buf[batch_of(e)] = acc_ref[lax.rem(e, G)].astype(o_buf.dtype)
            acc_ref[lax.rem(e, G)] = jnp.zeros(acc_ref.shape[1:], F32)

        return carry

    lax.fori_loop(0, N - 2, iteration, 0)

    todo = list(range(VA, NP))
    v_last = v_cp(i32(N - 1))

    def tail_tick_x(name):
        for prio in (0, 1, 0, 1):
            if todo:
                piece(v_last, todo.pop(0), prio)

    def tail_tick_y(name):
        if name == "y9":
            o_buf[B - 1, pl.ds(0, RG), pl.ds(0, Dh)] = (
                op_ref[(N - 1) % NS, 0, pl.ds(0, RG), :].astype(o_buf.dtype))
            o_cp(0, B - G, 0).start(priority=1)

    def no_tick(name):
        pass

    wait_k(i32(N - 1))
    stage_x(i32(N - 1), tail_tick_x, with_q=False)
    assert not todo
    for g in range(Sq // RG):
        c_group(i32(N - 1), g, KP, [0])
    wait_v(i32(N - 2))
    stage_y(i32(N - 2), tail_tick_y)
    for g in range(Sq // RG):
        c_group(i32(N - 1), g, KP, [1])
    wait_v(i32(N - 1))
    last = []

    def finish_batch(e, o):
        a = len(last) // 2
        for c0, cc in ((0, 256), (256, D - 256)):
            cols = pl.ds(c0, cc)
            y = lax.dot_general(o, wot_buf[cols, hcol(e)], NT, preferred_element_type=F32)
            o_buf[B - G + a, :, cols] = (acc_ref[a, :, cols] + y).astype(o_buf.dtype)
            last.append(pltpu.make_async_copy(
                o_buf.at[B - G + a, :, cols], o_hbm.at[B - G + a, :, cols], osem.at[1 + len(last)]))
            last[-1].start(priority=0)

    stage_y(i32(N - 1), no_tick, KP, finish_batch)
    finish_batch(i32(N - 1), merge(i32(N - 1)))
    o_cp(0, B - G, 0).wait()
    for c in last:
        c.wait()


@jax.jit
def pallas_standalone__mha_block_cached__near_ridge_kernel(
    x: jax.Array,
    k_cache: jax.Array,
    v_cache: jax.Array,
    wq: jax.Array,
    wo: jax.Array,
):
    B, Sq, D = x.shape
    _, H, Sk, Dh = k_cache.shape
    assert Sk == NR * RR and Dh == 256 and B % G == 0 and Sq % RG == 0
    assert H * Dh > WT1 * 128 and D % (8 * NR) == 0 and D > 256 and B > G
    assert (B * Sq) % 64 == 0 and (B * Sq) // 32 >= NP
    in_hbm = pl.BlockSpec(memory_space=pl.ANY)
    kv_shape = (B * H * NR // G, RR * G, Dh)
    return pl.pallas_call(
        _kernel,
        in_specs=[in_hbm] * 5,
        out_specs=in_hbm,
        out_shape=jax.ShapeDtypeStruct((B, Sq, D), x.dtype),
        scratch_shapes=[
            pltpu.VMEM((B * Sq, D), BF16),
            pltpu.VMEM((D, H * Dh), BF16),
            pltpu.VMEM((D, H * Dh), BF16),
            pltpu.VMEM((NPLANES, RR, Dh), BF16),
            pltpu.VMEM((NS, Sq, Dh), BF16),
            pltpu.VMEM((Sq, Sk), F32),
            pltpu.VMEM((NS, G, Sq, 128), F32),
            pltpu.VMEM((NS, G, Sq, 128), F32),
            pltpu.VMEM((NS, G, Sq, Dh), F32),
            pltpu.VMEM((G, Sq, D), F32),
            pltpu.VMEM((B, Sq, D), BF16),
            pltpu.SemaphoreType.DMA((NKB,)),
            pltpu.SemaphoreType.DMA((NVB,)),
            pltpu.SemaphoreType.DMA((3,)),
            pltpu.SemaphoreType.DMA((5,)),
        ],
        compiler_params=pltpu.CompilerParams(
            vmem_limit_bytes=64 * 1024 * 1024, disable_bounds_checks=True),
    )(x.reshape(B * Sq, D), k_cache.reshape(kv_shape), v_cache.reshape(kv_shape), wq, wo.T)
```
